```python
import jax
import jax.numpy as jnp

def _softmax(x, axis=-1):
    return jax.nn.softmax(x, axis=axis)

def _gelu(x):
    return jax.nn.gelu(x, approximate=True)

def _silu(x):
    return jax.nn.silu(x)

def _sigmoid(x):
    return jax.nn.sigmoid(x)

def _layernorm(x, axis=-1, eps=1e-05):
    m = jnp.mean(x, axis=axis, keepdims=True)
    v = jnp.var(x, axis=axis, keepdims=True)
    return (x - m) / jnp.sqrt(v + eps)

def _scatter_add(tgt, idx, src, axis=0):
    return tgt.at[idx].add(src)

def _segment_sum(src, seg, n):
    return jax.ops.segment_sum(src, seg, n)

class _Rng:

    def __init__(self, key):
        self._k = key

    def _next(self):
        self._k, sub = jax.random.split(self._k)
        return sub

    def normal(self, shape):
        return jax.random.normal(self._next(), shape, dtype=jnp.bfloat16)

    def randint(self, lo, hi, shape):
        return jax.random.randint(self._next(), shape, lo, hi, dtype=jnp.int32)

    def uniform(self, shape, lo=0.0, hi=1.0):
        return jax.random.uniform(self._next(), shape, jnp.bfloat16, lo, hi)

    def permutation(self, n):
        return jax.random.permutation(self._next(), n)
kernel_name = 'interleave_layers__memory_aug_infini_attn__moe_arch_mod__prompt'

def setup_inputs():
    _rng = _Rng(jax.random.key(int.from_bytes(__import__("os").urandom(4), "little")))
    _w = lambda a: (lambda t: t.astype(jnp.bfloat16) if jnp.issubdtype(t.dtype, jnp.floating) else t)(jnp.asarray(a))

    def _A_setup():
        B, S, D, H = (1, 2048, 1024, 32)
        N = 4
        L = max(1, S // N)
        sc = D ** (-0.5)
        return {'x': _w((lambda *s: _rng.normal(s) * 0.05)(B, N * L, D)), 'wq': _w((lambda *s: _rng.normal(s) * 0.05)(D, D) * sc), 'wk': _w((lambda *s: _rng.normal(s) * 0.05)(D, D) * sc), 'wv': _w((lambda *s: _rng.normal(s) * 0.05)(D, D) * sc), 'wo': _w((lambda *s: _rng.normal(s) * 0.05)(D, D) * sc), 'beta': _w((lambda *s: _rng.normal(s) * 0.05)(H))}
    _A_in = _A_setup()

    def _B_setup():
        B, S, D, F, C = (1, 2048, 1024, 3584, 2)
        return {'x': _w((lambda *s: _rng.normal(s) * 0.05)(B, S, D)), 'w_r': _w((lambda *s: _rng.normal(s) * 0.05)(D)), 'w_gate': _w((lambda *s: _rng.normal(s) * 0.05)(D, F)), 'w_up': _w((lambda *s: _rng.normal(s) * 0.05)(D, F)), 'w_down': _w((lambda *s: _rng.normal(s) * 0.05)(F, D))}
    _B_in = _B_setup()
    return {'A_x': _A_in['x'], 'A_wq': _A_in['wq'], 'A_wk': _A_in['wk'], 'A_wv': _A_in['wv'], 'A_wo': _A_in['wo'], 'A_beta': _A_in['beta'], 'B_x': _B_in['x'], 'B_w_r': _B_in['w_r'], 'B_w_gate': _B_in['w_gate'], 'B_w_up': _B_in['w_up'], 'B_w_down': _B_in['w_down']}

def reference(A_x, A_wq, A_wk, A_wv, A_wo, A_beta, B_x, B_w_r, B_w_gate, B_w_up, B_w_down):

    def _A_ref(x, wq, wk, wv, wo, beta):
        B, S, D = x.shape
        H = 32
        Dh = D // H
        N = 4
        L = S // N
        q = (lambda x, *d: x.transpose(*d))((x @ wq).reshape(B, S, H, Dh), 0, 2, 1, 3).reshape(B, H, N, L, Dh)
        k = (lambda x, *d: x.transpose(*d))((x @ wk).reshape(B, S, H, Dh), 0, 2, 1, 3).reshape(B, H, N, L, Dh)
        v = (lambda x, *d: x.transpose(*d))((x @ wv).reshape(B, S, H, Dh), 0, 2, 1, 3).reshape(B, H, N, L, Dh)
        phi = lambda t: jnp.where(t > 0, t + 1.0, jnp.exp(t))
        scale = Dh ** (-0.5)
        ar = jnp.arange(L)
        mask = (lambda x, dt: x.astype(dt))(ar[:, None] < ar[None, :], x.dtype) * -1000000000.0
        g = _sigmoid(beta).reshape(1, H, 1, 1)
        M = jnp.einsum('bhd,bhe->bhde', q[:, :, 0, 0, :] * 0.0, q[:, :, 0, 0, :] * 0.0)
        z = q[:, :, 0, 0, :] * 0.0
        outs = []
        for s in range(N):
            qs, ks, vs = (q[:, :, s].copy(), k[:, :, s].copy(), v[:, :, s].copy())
            logits = jnp.einsum('bhqd,bhkd->bhqk', qs, ks) * scale + mask
            p = _softmax(logits, axis=-1)
            a_dot = jnp.einsum('bhqk,bhkd->bhqd', p, vs)
            pq = phi(qs)
            num = jnp.einsum('bhld,bhde->bhle', pq, M)
            den = jnp.einsum('bhld,bhd->bhl', pq, z)[..., None] + 1e-06
            a_mem = num / den
            o = g * a_mem + (1.0 - g) * a_dot
            outs.append(o)
            pk = phi(ks)
            M = M + jnp.einsum('bhld,bhle->bhde', pk, vs)
            z = z + jnp.einsum('bhld->bhd', pk)
        o = (lambda x, *d: x.transpose(*d))(jnp.stack(outs, 2).reshape(B, H, S, Dh), 0, 2, 1, 3).reshape(B, S, D)
        return o @ wo

    def _B_ref(x, w_r, w_gate, w_up, w_down):
        B, S, D = x.shape
        C = 2
        r = x @ w_r
        idx = jnp.argsort(-r, axis=-1)[:, :C]
        idx_e = jnp.repeat(idx.reshape(B, C, 1), D, axis=2)
        x_sel = jnp.take_along_axis(x, idx_e, axis=1)
        g = _silu(x_sel @ w_gate)
        u = x_sel @ w_up
        y = g * u @ w_down
        r_sel = _sigmoid(jnp.take_along_axis(r, idx, axis=1))
        y = y * r_sel.reshape(B, C, 1)
        b_off = (jnp.arange(B) * S).reshape(B, 1)
        flat_idx = (idx + b_off).reshape(B * C)
        zero = (x * 0.0).reshape(B * S, D)
        upd = _scatter_add(zero, flat_idx, y.reshape(B * C, D), axis=0)
        return x + upd.reshape(B, S, D)
    x = A_x
    x = x + _A_ref(_layernorm(x, axis=-1), A_wq, A_wk, A_wv, A_wo, A_beta)
    x = x + _B_ref(_layernorm(x, axis=-1), B_w_r, B_w_gate, B_w_up, B_w_down)
    x = x + _A_ref(_layernorm(x, axis=-1), A_wq, A_wk, A_wv, A_wo, A_beta)
    x = x + _B_ref(_layernorm(x, axis=-1), B_w_r, B_w_gate, B_w_up, B_w_down)
    return x
```

```python
import math

import jax
import jax.numpy as jnp
import numpy as np
from jax import lax
import jax.experimental.pallas as pl
import jax.experimental.pallas.tpu as pltpu

S = 2048
D = 1024
H = 32
DH = 32
NSEG = 4
L = S // NSEG
G = 8
F = 3584
BR = 512

f32 = jnp.float32
bf16 = jnp.bfloat16
u32 = jnp.uint32

EPS_B = 1.0013580322265625e-05
SCALE_B = 0.1767578125
LOG2E = math.log2(math.e)
QSCALE = SCALE_B * LOG2E
NEG = -1e30

TILES = [(t, h, kt) for t in range(4) for h in range(4) for kt in range(t + 1)]
TIDX = {x: i for i, x in enumerate(TILES)}


def _rb(v):
    return v.astype(bf16).astype(f32)


def _pack(v):
    return pltpu.bitcast(v, u32)


def _unpack(v):
    return pltpu.bitcast(v, bf16)


def _ln(v):
    mean = jnp.mean(v, axis=-1, keepdims=True)
    d = v - mean
    var = jnp.mean(d * d, axis=-1, keepdims=True)
    den = _rb(jnp.sqrt(_rb(_rb(var) + EPS_B)))
    return (d * (1.0 / den)).astype(bf16)


def _phi(t):
    return jnp.where(t > 0, t + 1.0, jnp.exp(t))


def _nt_dot(a, b):
    return lax.dot_general(a, b, (((1,), (1,)), ((), ())), preferred_element_type=f32)


def _dot(a, b):
    return jnp.dot(a, b, preferred_element_type=f32)


def _kernel(x_hbm, wq_hbm, wk_hbm, wv_hbm, wo_hbm, beta_hbm, wr_hbm, wg_hbm, wu_hbm, wd_hbm,
            out_hbm,
            xb, wqk, wv, wo, wg, wu, wd, beta_v, wr_v,
            xres, xn, qk, pqk, vT, o_s, SA, SB, MA, MB, Mst, Lst, AA, AB, xn2, r_s,
            hm_s, cm_s, gate_s, one_s, patch, sems):
    def x_copy(s):
        return pltpu.make_async_copy(x_hbm.at[pl.ds(s * L, L)], xb.at[pl.ds(s * L, L)], sems.at[s])

    w_copies = [
        pltpu.make_async_copy(wq_hbm, wqk.at[0], sems.at[4]),
        pltpu.make_async_copy(wk_hbm, wqk.at[1], sems.at[5]),
        pltpu.make_async_copy(wv_hbm, wv, sems.at[6]),
        pltpu.make_async_copy(wo_hbm, wo, sems.at[7]),
        pltpu.make_async_copy(wg_hbm, wg, sems.at[8]),
        pltpu.make_async_copy(wu_hbm, wu, sems.at[9]),
        pltpu.make_async_copy(wd_hbm, wd, sems.at[10]),
        pltpu.make_async_copy(beta_hbm, beta_v, sems.at[11]),
        pltpu.make_async_copy(wr_hbm, wr_v, sems.at[12]),
    ]
    x_copy(0).start()
    w_copies[0].start()
    for s in range(1, NSEG):
        x_copy(s).start()
    for c in w_copies[1:]:
        c.start()

    lane8 = lax.broadcasted_iota(jnp.int32, (8, 128), 1)
    for h in range(4):
        hm_s[h] = jnp.where((lane8 >= 32 * h) & (lane8 < 32 * h + 32), jnp.uint32(0xFFFFFFFF), jnp.uint32(0))
    ki = lax.broadcasted_iota(jnp.int32, (128, 128), 0)
    qi = lax.broadcasted_iota(jnp.int32, (128, 128), 1)
    cm_s[...] = jnp.where(ki <= qi, 0.0, NEG).astype(f32)
    row16 = lax.broadcasted_iota(jnp.int32, (16, 128), 0)
    one_s[...] = _pack(jnp.where(row16 == 0, 1.0, 0.0).astype(bf16))

    w_copies[7].wait()
    w_copies[8].wait()
    gate_row = jax.nn.sigmoid(beta_v[...].astype(f32).reshape(1, H))
    gate_row = jnp.broadcast_to(gate_row, (8, H))
    lane_h = lax.broadcasted_iota(jnp.int32, (8, H), 1)
    for h in range(H):
        gh = jnp.sum(jnp.where(lane_h == h, gate_row, 0.0), axis=-1, keepdims=True)
        gate_s[h] = jnp.broadcast_to(gh, (8, 128))
    wr_row = wr_v[...].astype(f32).reshape(1, D)

    for s in range(NSEG):
        x_copy(s).wait()

        def ln0(j, _, s=s):
            r0 = pl.multiple_of(s * L + j * 16, 16)
            v = xb[pl.ds(r0, 16), :].astype(f32)
            xres[pl.ds(r0, 16), :] = v
            xn[pl.ds(pl.multiple_of(s * (L // 2) + j * 8, 8), 8), :] = _pack(_ln(v))

        lax.fori_loop(0, L // 16, ln0, None, unroll=4)

    for c in w_copies[:4]:
        c.wait()

    def out_copy(b):
        return pltpu.make_async_copy(xb.at[pl.ds(b * BR, BR)], out_hbm.at[pl.ds(b * BR, BR)], sems.at[13 + b])

    def layer(l, _):
        def qk_body(i, _):
            which = i // NSEG
            s = i % NSEG
            xs = _unpack(xn[pl.ds(pl.multiple_of(s * (L // 2), L // 2), L // 2), :])
            y = _dot(xs, wqk[which])
            c = jnp.where(which == 0, QSCALE, 1.0).astype(f32)
            ys = _pack((y * c).astype(bf16))
            ps = _pack(_phi(y).astype(bf16))
            r0 = pl.multiple_of(s * (L // 2), L // 2)
            for g in range(G):
                qk[which, g, pl.ds(r0, L // 2), :] = ys[:, 128 * g:128 * (g + 1)]
                pqk[which, g, pl.ds(r0, L // 2), :] = ps[:, 128 * g:128 * (g + 1)]

        lax.fori_loop(0, 2 * NSEG, qk_body, None)

        def v_body(s, _):
            xs = _unpack(xn[pl.ds(pl.multiple_of(s * (L // 2), L // 2), L // 2), :])
            y = _dot(xs, wv[...]).astype(bf16)
            for g in range(G):
                vT[g, s] = _pack(y[:, 128 * g:128 * (g + 1)].T)

        lax.fori_loop(0, NSEG, v_body, None)

        Mst[...] = jnp.zeros(Mst.shape, f32)
        Lst[...] = jnp.zeros(Lst.shape, u32)

        def step(i_qk, i_sm, Sw, Mw, Sr, Mr, doqk=True, dosm=True):
            sq, gq = i_qk // G, i_qk % G
            ss, gs = i_sm // G, i_sm % G
            rq = pl.multiple_of(sq * (L // 2), L // 2)
            rs = pl.multiple_of(ss * (L // 2), L // 2)
            M = {}
            O = {}
            LS = {}
            REC = {}

            def qk_tile(t, h, kt):
                kk = qk[1, gq, pl.ds(rq + 64 * kt, 64), :]
                qt = _unpack(qk[0, gq, pl.ds(rq + 64 * t, 64), :])
                km = _unpack(kk & hm_s[h][0:1, :])
                sc = _nt_dot(km, qt)
                if kt == t:
                    sc = sc + cm_s[...]
                Sw[TIDX[t, h, kt]] = sc
                mm = jnp.max(sc.reshape(16, 8, 128), axis=0)
                M[t, h] = mm if kt == 0 else jnp.maximum(M[t, h], mm)
                if kt == t:
                    Mw[4 * t + h] = jnp.broadcast_to(jnp.max(M[t, h], axis=0, keepdims=True), (8, 128))

            def sm_tile(t, h, kt):
                if h == 0 and kt == 0:
                    pq = _unpack(pqk[0, gs, pl.ds(rs + 64 * t, 64), :])
                    REC[t] = _nt_dot(_unpack(Lst[gs]), pq)
                sc = Sr[TIDX[t, h, kt]]
                m = Mr[4 * t + h]
                p = jnp.exp2(sc.reshape(16, 8, 128) - m[None]).reshape(128, 128)
                ls = jnp.sum(p.reshape(16, 8, 128), axis=0)
                vt = _unpack(vT[gs, ss, 16 * h:16 * h + 16, 128 * kt:128 * kt + 128])
                o = _dot(vt, p.astype(bf16))
                if kt == 0:
                    O[t, h] = o
                    LS[t, h] = ls
                else:
                    O[t, h] = O[t, h] + o
                    LS[t, h] = LS[t, h] + ls
                if kt == t and h == 3:
                    rec = REC[t]
                    rden = 1.0 / (rec[128:136] + 1e-6)
                    rows = []
                    for hh in range(4):
                        gt = gate_s[4 * gs + hh][0:1, :]
                        lsum = jnp.sum(LS[t, hh], axis=0, keepdims=True)
                        c1 = gt * rden[hh:hh + 1, :]
                        c2 = (1.0 - gt) * (1.0 / lsum)
                        rows.append(rec[32 * hh:32 * hh + 32] * c1 + O[t, hh] * c2)
                    ot = jnp.concatenate(rows, axis=0).astype(bf16)
                    o_s[gs, pl.ds(rs + 64 * t, 64), :] = _pack(ot.T)

            for x in TILES:
                if dosm:
                    sm_tile(*x)
                if doqk:
                    qk_tile(*x)
            if dosm:
                lhs = jnp.concatenate(
                    [_unpack(vT[gs, ss]), jnp.concatenate([_unpack(one_s[...])] * 4, axis=1)], axis=0)
                pk = _unpack(pqk[1, gs, pl.ds(rs, L // 2), :])
                upd = _dot(lhs, pk)
                mn = Mst[gs] + upd[0:136]
                Mst[gs] = mn
                hmask = jnp.concatenate([hm_s[hh] for hh in range(4) for _ in range(4)], axis=0)
                mb = pltpu.bitcast(pltpu.bitcast(mn[0:128], u32) & hmask, f32)
                sub = lax.broadcasted_iota(jnp.int32, (16, 128), 0)
                lane = lax.broadcasted_iota(jnp.int32, (16, 128), 1)
                z = jnp.broadcast_to(mn[128:129], (16, 128))
                zb = jnp.where(lane // 32 == sub, z, 0.0)
                Lst[gs] = _pack(jnp.concatenate([mb, zb], axis=0).astype(bf16))

        step(0, 0, SB, MB, SA, MA, dosm=False)

        def att_body(i, _):
            nxt = jnp.minimum(i + 1, 4 * G - 1)

            @pl.when(i % 2 == 0)
            def _():
                step(nxt, i, SA, MA, SB, MB)

            @pl.when(i % 2 == 1)
            def _():
                step(nxt, i, SB, MB, SA, MA)

        lax.fori_loop(0, 4 * G, att_body, None)

        def oproj(b, A):
            r0 = pl.multiple_of(b * (BR // 2), BR // 2)
            o = jnp.concatenate([_unpack(o_s[g, pl.ds(r0, BR // 2), :]) for g in range(G)], axis=1)
            A[...] = _dot(o, wo[...])

        def epilogue(b, A):
            lane = lax.broadcasted_iota(jnp.int32, (8, 128), 1)
            racc = jnp.zeros((8, 128), f32)
            for j in range(BR // 16):
                r0 = pl.multiple_of(b * BR + j * 16, 16)
                p0 = pl.multiple_of(b * (BR // 2) + j * 8, 8)
                x1 = _rb(xres[pl.ds(r0, 16), :] + _rb(A[j * 16:(j + 1) * 16, :]))
                n2b = _ln(x1)
                xn2[pl.ds(p0, 8), :] = _pack(n2b)
                n2 = n2b.astype(f32)
                r = jnp.sum(n2 * wr_row, axis=-1, keepdims=True)
                base = (b % 2) * (BR // 8) + 2 * j
                racc = jnp.where(lane == base, r[0:8], racc)
                racc = jnp.where(lane == base + 1, r[8:16], racc)
                x2b = (x1 + n2).astype(bf16)
                x2 = x2b.astype(f32)
                xres[pl.ds(r0, 16), :] = x2
                xb[pl.ds(r0, 16), :] = x2b
                xn[pl.ds(p0, 8), :] = _pack(_ln(x2))
            half = b // 2

            @pl.when(b % 2 == 0)
            def _():
                r_s[half] = racc

            @pl.when(b % 2 == 1)
            def _():
                r_s[half] = r_s[half] + racc

        NB = S // BR
        oproj(0, AA)

        def op_body(i, _):
            @pl.when((l == 1) & (i >= 2))
            def _():
                out_copy(i - 2).start()

            @pl.when(i % 2 == 1)
            def _():
                oproj(i, AB)
                epilogue(i - 1, AA)

            @pl.when(i % 2 == 0)
            def _():
                oproj(i, AA)
                epilogue(i - 1, AB)

        lax.fori_loop(1, NB, op_body, None)

        @pl.when(l == 1)
        def _():
            out_copy(NB - 2).start()

        epilogue(NB - 1, AB if (NB - 1) % 2 == 1 else AA)

        @pl.when(l == 1)
        def _():
            out_copy(NB - 1).start()

        @pl.when(l == 0)
        def _():
            for c in w_copies[4:7]:
                c.wait()

        rr = _rb(jnp.concatenate([r_s[0], r_s[1]], axis=0))
        sub = lax.broadcasted_iota(jnp.int32, (16, 128), 0)
        lane = lax.broadcasted_iota(jnp.int32, (16, 128), 1)
        pos = (sub // 8) * 1024 + lane * 8 + (sub % 8)
        m1 = jnp.max(rr)
        i1 = jnp.min(jnp.where(rr == m1, pos, S))
        rr2 = jnp.where(pos == i1, -jnp.inf, rr)
        m2 = jnp.max(rr2)
        i2 = jnp.min(jnp.where(rr2 == m2, pos, S))
        i1 = jnp.clip(i1, 0, S - 1)
        i2 = jnp.clip(i2, 0, S - 1)

        row = lax.broadcasted_iota(jnp.int32, (16, D), 0)

        def pick(i):
            blk = _unpack(xn2[pl.ds(pl.multiple_of((i // 16) * 8, 8), 8), :]).astype(f32)
            return jnp.sum(jnp.where(row == i % 16, blk, 0.0), axis=0, keepdims=True)

        xs = jnp.where(row == 0, pick(i1), jnp.where(row == 1, pick(i2), 0.0)).astype(bf16)
        y = jnp.zeros((16, D), f32)
        FC = 512
        for c in range(F // FC):
            gg = _rb(_dot(xs, wg[:, c * FC:(c + 1) * FC]))
            uu = _rb(_dot(xs, wu[:, c * FC:(c + 1) * FC]))
            a = (_rb(gg * jax.nn.sigmoid(gg)) * uu).astype(bf16)
            y = y + _dot(a, wd[c * FC:(c + 1) * FC, :])
        rsel = jnp.where(row == 0, m1, m2)
        upd = _rb(_rb(y) * _rb(jax.nn.sigmoid(rsel)))

        def fix(i, j, slot):
            r0 = pl.multiple_of((i // 16) * 16, 16)
            xv = xres[pl.ds(r0, 16), :]
            xv = _rb(xv + jnp.where(row == i % 16, upd[j:j + 1, :], 0.0))
            xres[pl.ds(r0, 16), :] = xv
            xn[pl.ds(pl.multiple_of((i // 16) * 8, 8), 8), :] = _pack(_ln(xv))
            patch[slot] = xv.astype(bf16)

        fix(i1, 0, 0)
        fix(i2, 1, 1)

        @pl.when(l == 1)
        def _():
            for b in range(NB):
                out_copy(b).wait()
            b1 = pl.multiple_of((i1 // 16) * 16, 16)
            b2 = pl.multiple_of((i2 // 16) * 16, 16)
            c1 = pltpu.make_async_copy(patch.at[0], out_hbm.at[pl.ds(b1, 16)], sems.at[17])
            c2 = pltpu.make_async_copy(patch.at[1], out_hbm.at[pl.ds(b2, 16)], sems.at[18])

            @pl.when(b1 != b2)
            def _():
                c1.start()

            c2.start()

            @pl.when(b1 != b2)
            def _():
                c1.wait()

            c2.wait()

    lax.fori_loop(0, 2, layer, None)


@jax.jit
def pallas_interleave_layers__memory_aug_infini_attn__moe_arch_mod__prompt_kernel(
    A_x, A_wq, A_wk, A_wv, A_wo, A_beta, B_x, B_w_r, B_w_gate, B_w_up, B_w_down,
):
    del B_x
    x = A_x.reshape(S, D)
    hbm = pl.BlockSpec(memory_space=pltpu.HBM)
    scratch = [
        pltpu.VMEM((S, D), bf16),
        pltpu.VMEM((2, D, D), bf16),
        pltpu.VMEM((D, D), bf16),
        pltpu.VMEM((D, D), bf16),
        pltpu.VMEM((D, F), bf16),
        pltpu.VMEM((D, F), bf16),
        pltpu.VMEM((F, D), bf16),
        pltpu.VMEM((H,), bf16),
        pltpu.VMEM((D,), bf16),
        pltpu.VMEM((S, D), f32),
        pltpu.VMEM((S // 2, D), u32),
        pltpu.VMEM((2, G, S // 2, 128), u32),
        pltpu.VMEM((2, G, S // 2, 128), u32),
        pltpu.VMEM((G, NSEG, 64, L), u32),
        pltpu.VMEM((G, S // 2, 128), u32),
        pltpu.VMEM((40, 128, 128), f32),
        pltpu.VMEM((40, 128, 128), f32),
        pltpu.VMEM((16, 8, 128), f32),
        pltpu.VMEM((16, 8, 128), f32),
        pltpu.VMEM((G, 136, 128), f32),
        pltpu.VMEM((G, 72, 128), u32),
        pltpu.VMEM((BR, D), f32),
        pltpu.VMEM((BR, D), f32),
        pltpu.VMEM((S // 2, D), u32),
        pltpu.VMEM((2, 8, 128), f32),
        pltpu.VMEM((4, 8, 128), u32),
        pltpu.VMEM((128, 128), f32),
        pltpu.VMEM((H, 8, 128), f32),
        pltpu.VMEM((8, 128), u32),
        pltpu.VMEM((2, 16, D), bf16),
        pltpu.SemaphoreType.DMA((19,)),
    ]
    out = pl.pallas_call(
        _kernel,
        out_shape=jax.ShapeDtypeStruct((S, D), bf16),
        in_specs=[hbm] * 10,
        out_specs=hbm,
        scratch_shapes=scratch,
        compiler_params=pltpu.CompilerParams(vmem_limit_bytes=110 * 1024 * 1024),
        name="infini_mod_kernel",
    )(x, A_wq, A_wk, A_wv, A_wo, A_beta, B_w_r, B_w_gate, B_w_up, B_w_down)
    return out.reshape(1, S, D)
```

```python
import math

import jax
import jax.numpy as jnp
from jax import lax
import jax.experimental.pallas as pl
import jax.experimental.pallas.tpu as pltpu

S = 2048
D = 1024
H = 32
DH = 32
NSEG = 4
L = S // NSEG
G = 8
F = 3584
BR = 512
NB = S // BR
NI = 4
SKEW = 8
TIE0, TIE1 = 600, 8150
FC = 512
NC = F // FC
NLAYERS = 2

f32 = jnp.float32
bf16 = jnp.bfloat16
u32 = jnp.uint32

EPS_B = 1.0013580322265625e-05
SCALE_B = 0.1767578125
LOG2E = math.log2(math.e)
QSCALE = SCALE_B * LOG2E
NEG = -1e30

TILES = [(t, h, kt) for t in range(4) for h in range(4) for kt in range(t + 1)]
TIDX = {x: i for i, x in enumerate(TILES)}


def _rb(v):
    return v.astype(bf16).astype(f32)


def _pack(v):
    return pltpu.bitcast(v, u32)


def _unpack(v):
    return pltpu.bitcast(v, bf16)


def _rcp(v):
    y = pltpu.reciprocal(v, approx=True)
    return y * (2.0 - v * y)


def _inv_std(var):
    return _rcp(_rb(jnp.exp2(0.5 * jnp.log2(_rb(_rb(var) + EPS_B)))))


def _ln(v):
    d = v - jnp.mean(v, axis=-1, keepdims=True)
    return (d * _inv_std(jnp.mean(d * d, axis=-1, keepdims=True))).astype(bf16)


def _after(v):
    return jnp.where(v != v, jnp.uint32(1), jnp.uint32(0)) & jnp.uint32(0x10)


def _tie(p, v, dep):
    parts = [p[:8 * v]] if v else []
    parts.append(p[8 * v:8 * v + 8] | dep)
    if 8 * v + 8 < p.shape[0]:
        parts.append(p[8 * v + 8:])
    return jnp.concatenate(parts, axis=0) if len(parts) > 1 else parts[0]


def _phi(t):
    return jnp.where(t > 0, t + 1.0, jnp.exp(t))


def _nt_dot(a, b):
    return lax.dot_general(a, b, (((1,), (1,)), ((), ())), preferred_element_type=f32)


def _dot(a, b):
    return jnp.dot(a, b, preferred_element_type=f32)


def _cols(ref, c0, n, rows=slice(None)):
    return jnp.concatenate([ref[c, rows, :] for c in range(c0, c0 + n)], axis=1)


def _spread(deps, t0, t1):
    ties = {}
    for j, dep in enumerate(deps):
        when = t0 + (j * (t1 - t0)) // (len(deps) - 1)
        slot = ties.setdefault(when // 1024, {})
        key = (4 * ((when % 1024) // 512), (when % 512) // 16)
        slot[key] = dep if key not in slot else slot[key] | dep
    return ties


def _kernel(x_hbm, wq_hbm, wk_hbm, wv_hbm, wo_hbm, beta_hbm, wr_hbm, wg_hbm, wu_hbm, wd_hbm,
            out_hbm,
            xb, wq, wk, wv, wo, wg, wu, wd, beta_v, wr_v,
            xres, xn, qk, pqk, vT, o_s, SA, SB, MA, MB, Mst, Lst, AA, AB, xn2, r_s,
            hm_s, cm_s, gate_s, one_s, patch, stat_s, sems):
    def x_copy(s):
        r = pl.ds(pl.multiple_of(s * L, L), L)
        return pltpu.make_async_copy(x_hbm.at[r], xb.at[r], sems.at[s])

    def w_copies(src, dst, sem, c0=0, c1=None):
        c1 = dst.shape[0] if c1 is None else c1
        return [pltpu.make_async_copy(src.at[:, pl.ds(128 * c, 128)], dst.at[c], sems.at[sem])
                for c in range(c0, c1)]

    def start(copies):
        for c in copies:
            c.start()

    def wait(copies):
        for c in copies:
            c.wait()

    beta_c = pltpu.make_async_copy(beta_hbm, beta_v, sems.at[4])
    wr_c = pltpu.make_async_copy(wr_hbm, wr_v, sems.at[4])
    wq_lo, wq_hi = w_copies(wq_hbm, wq, 5, 0, 4), w_copies(wq_hbm, wq, 6, 4, 8)
    wk_c, wv_c, wo_c = w_copies(wk_hbm, wk, 7), w_copies(wv_hbm, wv, 8), w_copies(wo_hbm, wo, 9)
    mlp_c = w_copies(wg_hbm, wg, 10) + w_copies(wu_hbm, wu, 10) + w_copies(wd_hbm, wd, 10)

    beta_c.start()
    wr_c.start()
    x_copy(0).start()
    start(wq_lo)
    start(wq_hi)

    lane8 = lax.broadcasted_iota(jnp.int32, (8, 128), 1)
    for h in range(4):
        hm_s[h] = jnp.where((lane8 >= 32 * h) & (lane8 < 32 * h + 32), jnp.uint32(0xFFFFFFFF), jnp.uint32(0))
    ki = lax.broadcasted_iota(jnp.int32, (128, 128), 0)
    qi = lax.broadcasted_iota(jnp.int32, (128, 128), 1)
    cm_s[...] = jnp.where(ki <= qi, 0.0, NEG).astype(f32)
    row16 = lax.broadcasted_iota(jnp.int32, (16, 128), 0)
    one_s[...] = _pack(jnp.where(row16 == 0, 1.0, 0.0).astype(bf16))

    beta_c.wait()
    wr_c.wait()
    gate_row = jnp.broadcast_to(jax.nn.sigmoid(beta_v[...].astype(f32).reshape(1, H)), (8, H))
    lane_h = lax.broadcasted_iota(jnp.int32, (8, H), 1)
    for h in range(H):
        gh = jnp.sum(jnp.where(lane_h == h, gate_row, 0.0), axis=-1, keepdims=True)
        gate_s[h] = jnp.broadcast_to(gh, (8, 128))
    wr_row = wr_v[...].astype(f32).reshape(1, D)

    def first_ln(s, dst):
        xsub = xb.at[pl.ds(s * L, L)]
        rsub = xres.at[pl.ds(s * L, L)]
        nsub = dst.at[pl.ds(s * (L // 2), L // 2)]
        deps = []
        for j in range(L // 16):
            v = xsub[j * 16:(j + 1) * 16, :].astype(f32)
            rsub[j * 16:(j + 1) * 16, :] = v
            n = _pack(_ln(v))
            nsub[j * 8:(j + 1) * 8, :] = n
            deps.append(_after(pltpu.bitcast(n[:, 896:1024], f32)))
        return deps

    def out_copy(b):
        return pltpu.make_async_copy(xb.at[pl.ds(b * BR, BR)], out_hbm.at[pl.ds(b * BR, BR)], sems.at[11 + b])

    def proj_piece(src, s, w_ref, c, ties=None):
        xs = src.at[pl.ds(pl.multiple_of(s * (L // 2), L // 2), L // 2)]
        ps = [xs[:, 128 * g:128 * (g + 1)] for g in range(G)]
        for (g, v), dep in (ties or {}).items():
            ps[g] = _tie(ps[g], v, dep)
        return _dot(jnp.concatenate([_unpack(p) for p in ps], axis=1), w_ref[c])

    def qkv(src, s, hooks=None):
        r0 = pl.multiple_of(s * (L // 2), L // 2)
        ties = {}
        n = 0
        for which, w_ref in ((0, wq), (1, wk), (2, wv)):
            for g in range(G):
                if hooks and n in hooks:
                    ties = hooks[n]() or ties
                y = proj_piece(src, s, w_ref, g, ties.get(n))
                if which < 2:
                    qk.at[which, g, pl.ds(r0, L // 2)][...] = _pack(((y * QSCALE) if which == 0 else y).astype(bf16))
                    pqk.at[which, g, pl.ds(r0, L // 2)][...] = _pack(_phi(y).astype(bf16))
                else:
                    vT.at[g, s][...] = _pack(y.astype(bf16).T)
                n += 1

    def step(i_qk, i_sm, Sw, Mw, Sr, Mr, filler=None):
        if i_qk is not None:
            gq = pl.multiple_of(i_qk % G, NI)
            rq = pl.multiple_of((i_qk // G) * (L // 2), L // 2)
            q_q = qk.at[0, pl.ds(gq, NI), pl.ds(rq, L // 2)]
            q_k = qk.at[1, pl.ds(gq, NI), pl.ds(rq, L // 2)]
        if i_sm is not None:
            gs = pl.multiple_of(i_sm % G, NI)
            ss = i_sm // G
            rs = pl.multiple_of(ss * (L // 2), L // 2)
            s_pq = pqk.at[0, pl.ds(gs, NI), pl.ds(rs, L // 2)]
            s_pk = pqk.at[1, pl.ds(gs, NI), pl.ds(rs, L // 2)]
            s_v = vT.at[pl.ds(gs, NI), ss]
            s_o = o_s.at[pl.ds(gs, NI), pl.ds(rs, L // 2)]
            s_M = Mst.at[pl.ds(gs, NI)]
            s_L = Lst.at[pl.ds(gs, NI)]
            s_g = gate_s.at[pl.ds(4 * gs, 4 * NI)]
        M, O, LS, REC, UPD = {}, {}, {}, {}, {}

        def qk_tile(j, t, h, kt):
            kk = q_k[j, 64 * kt:64 * kt + 64, :]
            qt = _unpack(q_q[j, 64 * t:64 * t + 64, :])
            km = _unpack(kk & hm_s[h][0:1, :])
            sc = _nt_dot(km, qt)
            if kt == t:
                sc = sc + cm_s[...]
            Sw.at[40 * j + TIDX[t, h, kt]][...] = sc
            mm = jnp.max(sc.reshape(16, 8, 128), axis=0)
            M[t, h] = mm if kt == 0 else jnp.maximum(M[t, h], mm)
            if kt == t:
                Mw.at[16 * j + 4 * t + h][...] = jnp.broadcast_to(
                    jnp.max(M[t, h], axis=0, keepdims=True), (8, 128))

        def sm_tile(j, t, h, kt):
            if h == 0 and kt == 0:
                pq = _unpack(s_pq[j, 64 * t:64 * t + 64, :])
                REC[t] = _nt_dot(_unpack(s_L[j]), pq)
            sc = Sr[40 * j + TIDX[t, h, kt]]
            m = Mr[16 * j + 4 * t + h]
            p = jnp.exp2(sc.reshape(16, 8, 128) - m[None]).reshape(128, 128)
            ls = jnp.sum(p.reshape(16, 8, 128), axis=0)
            vt = _unpack(s_v[j, 16 * h:16 * h + 16, 128 * kt:128 * kt + 128])
            o = _dot(vt, p.astype(bf16))
            if kt == 0:
                O[t, h] = o
                LS[t, h] = ls
            else:
                O[t, h] = O[t, h] + o
                LS[t, h] = LS[t, h] + ls
            if kt == t:
                gt = s_g[4 * j + h][0:1, :]
                c2 = (1.0 - gt) * _rcp(jnp.sum(LS[t, h], axis=0, keepdims=True))
                O[t, h] = O[t, h] * c2
            if kt == t and h == 3:
                rec = REC[t]
                rden = _rcp(rec[128:136] + 1e-6)
                rows = []
                for hh in range(4):
                    c1 = s_g[4 * j + hh][0:1, :] * rden[hh:hh + 1, :]
                    rows.append(rec[32 * hh:32 * hh + 32] * c1 + O[t, hh])
                ot = jnp.concatenate(rows, axis=0).astype(bf16)
                s_o.at[j, pl.ds(64 * t, 64)][...] = _pack(ot.T)

        def mem_update_start(j):
            lhs = jnp.concatenate(
                [_unpack(s_v[j]), jnp.concatenate([_unpack(one_s[...])] * 4, axis=1)], axis=0)
            upd = _dot(lhs, _unpack(s_pk[j]))
            mn = s_M[j] + upd[0:136]
            s_M.at[j][...] = mn
            hmask = jnp.concatenate([hm_s[hh] for hh in range(4) for _ in range(4)], axis=0)
            mb = pltpu.bitcast(pltpu.bitcast(mn[0:128], u32) & hmask, f32)
            sub = lax.broadcasted_iota(jnp.int32, (16, 128), 0)
            lane = lax.broadcasted_iota(jnp.int32, (16, 128), 1)
            z = jnp.broadcast_to(mn[128:129], (16, 128))
            zb = jnp.where(lane // 32 == sub, z, 0.0)
            UPD[j] = _pack(jnp.concatenate([mb, zb], axis=0).astype(bf16))

        work = [(j, x) for j in range(NI) for x in TILES]
        n_sm = 0
        for n, (j, x) in enumerate(work):
            if i_sm is not None:
                target = len(work) if i_qk is None else min(len(work), ((n + 1) * len(work)) // (len(work) - SKEW) + 1)
                target = n + 1 if i_qk is None else target
                while n_sm < target:
                    js, xs_ = work[n_sm]
                    if xs_ == TILES[0]:
                        mem_update_start(js)
                    sm_tile(js, *xs_)
                    if xs_ == TILES[-1]:
                        s_L.at[js][...] = UPD[js]
                    n_sm += 1
            if i_qk is not None:
                qk_tile(j, *x)
            if filler is not None:
                filler(n + 1, len(work))

    def oproj_piece(b, A, c, ties=None):
        osub = o_s.at[:, pl.ds(pl.multiple_of(b * (BR // 2), BR // 2), BR // 2)]
        ps = [osub[g] for g in range(G)]
        for (g, v), dep in (ties or {}).items():
            ps[g] = _tie(ps[g], v, dep)
        o = jnp.concatenate([_unpack(p) for p in ps], axis=1)
        A[:, 128 * c:128 * (c + 1)] = _dot(o, wo[c])

    def epilogue_refs(b):
        return (xres.at[pl.ds(pl.multiple_of(b * BR, BR), BR)],
                xb.at[pl.ds(pl.multiple_of(b * BR, BR), BR)],
                xn2.at[pl.ds(pl.multiple_of(b * (BR // 2), BR // 2), BR // 2)],
                xn.at[pl.ds(pl.multiple_of(b * (BR // 2), BR // 2), BR // 2)])

    def epi1(refs, A, j, base, racc):
        xr, _, n2r, _ = refs
        rows = slice(j * 16, (j + 1) * 16)
        x1 = _rb(xr[rows, :] + A[rows, :])
        mean = jnp.mean(x1, axis=-1, keepdims=True)
        d = x1 - mean
        var = jnp.mean(d * d, axis=-1, keepdims=True)
        inv = _inv_std(var)
        n2b = (d * inv).astype(bf16)
        n2r[j * 8:(j + 1) * 8, :] = _pack(n2b)
        n2 = n2b.astype(f32)
        r = jnp.sum(n2 * wr_row, axis=-1, keepdims=True)
        lane = lax.broadcasted_iota(jnp.int32, (8, 128), 1)
        racc = jnp.where(lane == base + 2 * j, r[0:8], racc)
        racc = jnp.where(lane == base + 2 * j + 1, r[8:16], racc)
        grow = 1.0 + inv
        scale2 = grow * _inv_std(var * (grow * grow))
        done = _after(jnp.broadcast_to(r[0:8] + r[8:16], (8, 128)))
        return x1, mean, d, scale2, n2, racc, done

    def epi2(refs, j, x1, d, scale2, n2, last):
        xr, xo, _, n1r = refs
        rows = slice(j * 16, (j + 1) * 16)
        x2b = (x1 + n2).astype(bf16)
        x2 = x2b.astype(f32)
        xr[rows, :] = x2
        if last:
            xo[rows, :] = x2b
            return _after(x2[0:8, 896:1024])
        n1 = _pack((d * scale2).astype(bf16))
        n1r[j * 8:(j + 1) * 8, :] = n1
        return _after(pltpu.bitcast(n1[:, 896:1024], f32)) | _after(x2[0:8, 896:1024])

    def put_scores(b, racc):
        half = b // 2

        @pl.when(b % 2 == 0)
        def _():
            r_s[half] = racc

        @pl.when(b % 2 == 1)
        def _():
            r_s[half] = r_s[half] + racc

    def oproj_epilogue(b, A, bn, An, last):
        refs = epilogue_refs(b)
        racc = jnp.zeros((8, 128), f32)
        deps = []
        for j in range(BR // 16):
            x1, _, d, scale2, n2, racc, done = epi1(refs, A, j, (b % 2) * (BR // 8), racc)
            deps.append(done | epi2(refs, j, x1, d, scale2, n2, last))
        ties = _spread(deps, TIE0, TIE1)
        for c in range(G):
            oproj_piece(bn, An, c, ties.get(c))
        put_scores(b, racc)

    def layer(l):
        first, last = l == 0, l == NLAYERS - 1

        with jax.named_scope("P_qkv"):
            if first:
                bufs = (xn, xn2)
                x_copy(0).wait()
                x_copy(1).start()
                start(wk_c)
                start(wv_c)
                first_ln(0, bufs[0])
                wait(wq_lo)

                def after_q0():
                    wait(wk_c)
                    x_copy(1).wait()
                    x_copy(2).start()
                    x_copy(3).start()
                    return _spread(first_ln(1, bufs[1]), 8 * 1024 + 600, 16 * 1024 - 100)

                qkv(bufs[0], 0, {4: lambda: wait(wq_hi), 8: after_q0, 16: lambda: wait(wv_c)})
                for s in range(1, NSEG):
                    def before(s=s):
                        if s == 1:
                            start(wo_c)
                            start(mlp_c)
                        if s + 1 < NSEG:
                            x_copy(s + 1).wait()
                            return _spread(first_ln(s + 1, bufs[(s + 1) % 2]), 600, 16 * 1024)

                    qkv(bufs[s % 2], s, {0: before})
            else:
                lax.fori_loop(0, NSEG, lambda s, _: qkv(xn, s), None)

        Mst[...] = jnp.zeros(Mst.shape, f32)
        Lst[...] = jnp.zeros(Lst.shape, u32)
        nstep = 4 * G // NI
        with jax.named_scope("P_att"):
            step(0, None, SB, MB, None, None)

            def att_body(i, _):
                @pl.when(i % 2 == 0)
                def _():
                    step((i + 1) * NI, i * NI, SA, MA, SB, MB)

                @pl.when(i % 2 == 1)
                def _():
                    step((i + 1) * NI, i * NI, SB, MB, SA, MA)

            lax.fori_loop(0, nstep - 1, att_body, None)

        if first:
            wait(wo_c)

        def filler(n, total):
            if n % (total // G) == 0:
                oproj_piece(0, AA, n // (total // G) - 1)

        with jax.named_scope("P_op"):
            if (nstep - 1) % 2 == 0:
                step(None, (nstep - 1) * NI, None, None, SB, MB, filler)
            else:
                step(None, (nstep - 1) * NI, None, None, SA, MA, filler)

            def op_body(i, _):
                if last:
                    @pl.when(i >= 2)
                    def _():
                        out_copy(i - 2).start()

                @pl.when(i % 2 == 1)
                def _():
                    oproj_epilogue(i - 1, AA, i, AB, last)

                @pl.when(i % 2 == 0)
                def _():
                    oproj_epilogue(i - 1, AB, i, AA, last)

            lax.fori_loop(1, NB, op_body, None)

        if last:
            out_copy(NB - 2).start()

        with jax.named_scope("P_tail"):
            refs = epilogue_refs(NB - 1)
            A_last = AB if (NB - 1) % 2 == 1 else AA
            racc = jnp.zeros((8, 128), f32)
            for j in range(BR // 16):
                x1, mean, d, scale2, n2, racc, _ = epi1(refs, A_last, j, ((NB - 1) % 2) * (BR // 8), racc)
                if last:
                    epi2(refs, j, x1, d, scale2, n2, True)
                else:
                    A_last[j * 16:(j + 1) * 16, :] = x1
                    stat_s.at[0][j * 16:(j + 1) * 16, :] = jnp.broadcast_to(mean, (16, 128))
                    stat_s.at[1][j * 16:(j + 1) * 16, :] = jnp.broadcast_to(scale2, (16, 128))
            r_all = jnp.concatenate([r_s[0], r_s[1] + racc], axis=0)
            if last:
                out_copy(NB - 1).start()
            if first:
                wait(mlp_c)

            rr = pltpu.bitcast(_rb(r_all), u32)
            sub = lax.broadcasted_iota(jnp.int32, (16, 128), 0)
            lane = lax.broadcasted_iota(jnp.int32, (16, 128), 1)
            pos = ((sub // 8) * 1024 + lane * 8 + (sub % 8)).astype(u32)
            neg = (rr >> 31) == 1
            key = pltpu.bitcast(rr | jnp.where(neg, pos, (S - 1) - pos), f32)

            def top(k):
                return jnp.max(jnp.max(k, axis=1, keepdims=True), axis=0, keepdims=True)

            k1 = top(key)
            k2 = top(jnp.where(key == k1, -jnp.inf, key))

            def decode(k):
                kb = pltpu.bitcast(jnp.broadcast_to(k, (8, 128)), u32)
                code = kb & jnp.uint32(S - 1)
                p = jnp.where((kb >> 31) == 1, code, (S - 1) - code).astype(jnp.int32)
                score = pltpu.bitcast(kb & jnp.uint32(0xFFFF0000), f32)
                return jnp.clip(jnp.max(p), 0, S - 1), score

            i1, m1 = decode(k1)
            i2, m2 = decode(k2)

            row = lax.broadcasted_iota(jnp.int32, (16, D), 0)

            def pick(i):
                blk = _unpack(xn2[pl.ds(pl.multiple_of((i // 16) * 8, 8), 8), :]).astype(f32)
                return jnp.sum(jnp.where(row == i % 16, blk, 0.0), axis=0, keepdims=True)

            xs = jnp.where(row == 0, pick(i1), jnp.where(row == 1, pick(i2), 0.0)).astype(bf16)

            ties = {}
            if not last:
                for j in range(BR // 16):
                    rows = slice(j * 16, (j + 1) * 16)
                    x1 = A_last[rows, :]
                    n2 = _unpack(refs[2][j * 8:(j + 1) * 8, :]).astype(f32)
                    done = epi2(refs, j, x1, x1 - stat_s[0, rows, 0:1], stat_s[1, rows, 0:1], n2, False)
                    key_ = 3 + (j * (2 * NC - 3)) // (BR // 16)
                    ties[key_] = done if key_ not in ties else ties[key_] | done

            def weights(w_ref, c, key_):
                tiles = [_pack(w_ref[4 * c + t]) for t in range(4)] if key_ in ties else None
                if tiles is None:
                    return _cols(w_ref, 4 * c, 4)
                tiles[0] = _tie(tiles[0], 0, ties[key_])
                return jnp.concatenate([_unpack(t) for t in tiles], axis=1)

            def gate_up(c):
                gg = _rb(_dot(xs, weights(wg, c, 2 * c)))
                uu = _rb(_dot(xs, weights(wu, c, 2 * c + 1)))
                return (_rb(gg * jax.nn.sigmoid(gg)) * uu).astype(bf16)

            y = jnp.zeros((16, D), f32)
            a = gate_up(0)
            for c in range(NC):
                a_next = gate_up(c + 1) if c + 1 < NC else None
                y = y + _dot(a, _cols(wd, 0, G, slice(c * FC, (c + 1) * FC)))
                a = a_next
            row8 = lax.broadcasted_iota(jnp.int32, (16, 128), 0)
            gsel = _rb(jax.nn.sigmoid(jnp.where(row8 == 0, m1[0:1, :], m2[0:1, :])))
            upd = _rb(_rb(y) * jnp.concatenate([gsel] * (D // 128), axis=1))

            def rows_at(i):
                return pl.multiple_of((i // 16) * 16, 16)

            def updated(i0):
                xv = xres[pl.ds(rows_at(i0), 16), :]
                for i, j in ((i1, 0), (i2, 1)):
                    hit = (row == i % 16) & (i // 16 == i0 // 16)
                    xv = xv + jnp.where(hit, upd[j:j + 1, :], 0.0)
                return xv.astype(bf16)

            xv1, xv2 = updated(i1), updated(i2)
            if last:
                patch[0] = xv1
                patch[1] = xv2
                for b in range(NB):
                    out_copy(b).wait()
                b1, b2 = rows_at(i1), rows_at(i2)
                c1 = pltpu.make_async_copy(patch.at[0], out_hbm.at[pl.ds(b1, 16)], sems.at[15])
                c2 = pltpu.make_async_copy(patch.at[1], out_hbm.at[pl.ds(b2, 16)], sems.at[16])

                @pl.when(b1 != b2)
                def _():
                    c1.start()

                c2.start()

                @pl.when(b1 != b2)
                def _():
                    c1.wait()

                c2.wait()
            else:
                n1, n2 = _pack(_ln(xv1.astype(f32))), _pack(_ln(xv2.astype(f32)))
                for i, xv, nn in ((i1, xv1, n1), (i2, xv2, n2)):
                    xres[pl.ds(rows_at(i), 16), :] = xv.astype(f32)
                    xn.at[pl.ds(pl.multiple_of((i // 16) * 8, 8), 8)][...] = nn

    for l in range(NLAYERS):
        layer(l)


@jax.jit
def pallas_interleave_layers__memory_aug_infini_attn__moe_arch_mod__prompt_kernel(
    A_x, A_wq, A_wk, A_wv, A_wo, A_beta, B_x, B_w_r, B_w_gate, B_w_up, B_w_down,
):
    del B_x
    x = A_x.reshape(S, D)
    hbm = pl.BlockSpec(memory_space=pltpu.HBM)
    scratch = [
        pltpu.VMEM((S, D), bf16),
        pltpu.VMEM((D // 128, D, 128), bf16),
        pltpu.VMEM((D // 128, D, 128), bf16),
        pltpu.VMEM((D // 128, D, 128), bf16),
        pltpu.VMEM((D // 128, D, 128), bf16),
        pltpu.VMEM((F // 128, D, 128), bf16),
        pltpu.VMEM((F // 128, D, 128), bf16),
        pltpu.VMEM((D // 128, F, 128), bf16),
        pltpu.VMEM((H,), bf16),
        pltpu.VMEM((D,), bf16),
        pltpu.VMEM((S, D), f32),
        pltpu.VMEM((S // 2, D), u32),
        pltpu.VMEM((2, G, S // 2, 128), u32),
        pltpu.VMEM((2, G, S // 2, 128), u32),
        pltpu.VMEM((G, NSEG, 64, L), u32),
        pltpu.VMEM((G, S // 2, 128), u32),
        pltpu.VMEM((40 * NI, 128, 128), f32),
        pltpu.VMEM((40 * NI, 128, 128), f32),
        pltpu.VMEM((16 * NI, 8, 128), f32),
        pltpu.VMEM((16 * NI, 8, 128), f32),
        pltpu.VMEM((G, 136, 128), f32),
        pltpu.VMEM((G, 72, 128), u32),
        pltpu.VMEM((BR, D), f32),
        pltpu.VMEM((BR, D), f32),
        pltpu.VMEM((S // 2, D), u32),
        pltpu.VMEM((2, 8, 128), f32),
        pltpu.VMEM((4, 8, 128), u32),
        pltpu.VMEM((128, 128), f32),
        pltpu.VMEM((H, 8, 128), f32),
        pltpu.VMEM((8, 128), u32),
        pltpu.VMEM((2, 16, D), bf16),
        pltpu.VMEM((2, BR, 128), f32),
        pltpu.SemaphoreType.DMA((17,)),
    ]
    out = pl.pallas_call(
        _kernel,
        out_shape=jax.ShapeDtypeStruct((S, D), bf16),
        in_specs=[hbm] * 10,
        out_specs=hbm,
        scratch_shapes=scratch,
        compiler_params=pltpu.CompilerParams(vmem_limit_bytes=124 * 1024 * 1024),
        name="infini_mod_kernel",
    )(x, A_wq, A_wk, A_wv, A_wo, A_beta, B_w_r, B_w_gate, B_w_up, B_w_down)
    return out.reshape(1, S, D)
```

```python
import math

import jax
import jax.numpy as jnp
from jax import lax
import jax.experimental.pallas as pl
import jax.experimental.pallas.tpu as pltpu

S = 2048
D = 1024
H = 32
DH = 32
NSEG = 4
L = S // NSEG
G = 8
F = 3584
BR = 512
NB = S // BR
NI = 4
SKEW = 8
TIE0, TIE1 = 600, 8150
FC = 512
NC = F // FC
NLAYERS = 2

f32 = jnp.float32
bf16 = jnp.bfloat16
u32 = jnp.uint32

EPS_B = 1.0013580322265625e-05
SCALE_B = 0.1767578125
LOG2E = math.log2(math.e)
QSCALE = SCALE_B * LOG2E
NEG = -1e30

TILES = [(t, h, kt) for t in range(4) for h in range(4) for kt in range(t + 1)]
TIDX = {x: i for i, x in enumerate(TILES)}


def _rb(v):
    return v.astype(bf16).astype(f32)


def _pack(v):
    return pltpu.bitcast(v, u32)


def _unpack(v):
    return pltpu.bitcast(v, bf16)


def _rcp(v):
    y = pltpu.reciprocal(v, approx=True)
    return y * (2.0 - v * y)


def _inv_std(var):
    return _rcp(_rb(jnp.exp2(0.5 * jnp.log2(_rb(_rb(var) + EPS_B)))))


def _ln(v):
    d = v - jnp.mean(v, axis=-1, keepdims=True)
    return (d * _inv_std(jnp.mean(d * d, axis=-1, keepdims=True))).astype(bf16)


def _after(v):
    return jnp.where(v != v, jnp.uint32(1), jnp.uint32(0)) & jnp.uint32(0x10)


def _tie(p, v, dep):
    parts = [p[:8 * v]] if v else []
    parts.append(p[8 * v:8 * v + 8] | dep)
    if 8 * v + 8 < p.shape[0]:
        parts.append(p[8 * v + 8:])
    return jnp.concatenate(parts, axis=0) if len(parts) > 1 else parts[0]


def _phi(t):
    return jnp.where(t > 0, t + 1.0, jnp.exp(t))


def _nt_dot(a, b):
    return lax.dot_general(a, b, (((1,), (1,)), ((), ())), preferred_element_type=f32)


def _dot(a, b):
    return jnp.dot(a, b, preferred_element_type=f32)


def _wtile(ref, c, r0=0, nr=None):
    nr = ref.shape[1] if nr is None else nr
    return ref.bitcast(u32)[c, r0 // 2:(r0 + nr) // 2, :]


def _cols(ref, c0, n, r0=0, nr=None):
    return jnp.concatenate([_unpack(_wtile(ref, c, r0, nr)) for c in range(c0, c0 + n)], axis=1)


def _spread(deps, t0, t1):
    ties = {}
    for j, dep in enumerate(deps):
        when = t0 + (j * (t1 - t0)) // (len(deps) - 1)
        slot = ties.setdefault(when // 1024, {})
        key = (4 * ((when % 1024) // 512), (when % 512) // 16)
        slot[key] = dep if key not in slot else slot[key] | dep
    return ties


def _kernel(x_hbm, wq_hbm, wk_hbm, wv_hbm, wo_hbm, beta_hbm, wr_hbm, wg_hbm, wu_hbm, wd_hbm,
            out_hbm,
            xb, wq, wk, wv, wo, wg, wu, wd, beta_v, wr_v,
            xres, xn, qk, pqk, vT, o_s, SA, SB, MA, MB, Mst, Lst, AA, AB, xn2, r_s,
            hm_s, cm_s, gate_s, one_s, patch, stat_s, wr_s, zero_s, sems):
    def x_copy(s):
        r = pl.ds(pl.multiple_of(s * L, L), L)
        return pltpu.make_async_copy(x_hbm.at[r], xb.at[r], sems.at[s])

    def w_copies(src, dst, sem, c0=0, c1=None):
        c1 = dst.shape[0] if c1 is None else c1
        return [pltpu.make_async_copy(src.at[:, pl.ds(128 * c, 128)], dst.at[c], sems.at[sem])
                for c in range(c0, c1)]

    def start(copies):
        for c in copies:
            c.start()

    def wait(copies):
        for c in copies:
            c.wait()

    beta_c = pltpu.make_async_copy(beta_hbm, beta_v, sems.at[4])
    wr_c = pltpu.make_async_copy(wr_hbm, wr_v, sems.at[4])
    wq_lo, wq_mid, wq_hi = w_copies(wq_hbm, wq, 5, 0, 2), w_copies(wq_hbm, wq, 19, 2, 5), w_copies(wq_hbm, wq, 6, 5, 8)
    wk_c, wv_c, wo_c = w_copies(wk_hbm, wk, 7), w_copies(wv_hbm, wv, 8), w_copies(wo_hbm, wo, 9)
    mlp_c = w_copies(wg_hbm, wg, 10) + w_copies(wu_hbm, wu, 10) + w_copies(wd_hbm, wd, 10)

    def x0_copy(h):
        r = pl.ds(h * (L // 2), L // 2)
        return pltpu.make_async_copy(x_hbm.at[r], xb.at[r], sems.at[17 + h])

    beta_c.start()
    wr_c.start()
    x0_copy(0).start()
    x0_copy(1).start()
    start(wq_lo)
    start(wq_mid)
    start(wq_hi)
    start(wk_c)
    x_copy(1).start()
    start(wv_c)
    x_copy(2).start()
    x_copy(3).start()

    zero_s[0] = 0
    lane8 = lax.broadcasted_iota(jnp.int32, (8, 128), 1)
    for h in range(4):
        hm_s[h] = jnp.where((lane8 >= 32 * h) & (lane8 < 32 * h + 32), jnp.uint32(0xFFFFFFFF), jnp.uint32(0))
    ki = lax.broadcasted_iota(jnp.int32, (128, 128), 0)
    qi = lax.broadcasted_iota(jnp.int32, (128, 128), 1)
    cm_s[...] = jnp.where(ki <= qi, 0.0, NEG).astype(f32)
    row16 = lax.broadcasted_iota(jnp.int32, (16, 128), 0)
    one_s[...] = _pack(jnp.where(row16 == 0, 1.0, 0.0).astype(bf16))

    def setup_small():
        beta_c.wait()
        wr_c.wait()
        gate_row = jnp.broadcast_to(jax.nn.sigmoid(beta_v[...].astype(f32).reshape(1, H)), (8, H))
        lane_h = lax.broadcasted_iota(jnp.int32, (8, H), 1)
        for h in range(H):
            gh = jnp.sum(jnp.where(lane_h == h, gate_row, 0.0), axis=-1, keepdims=True)
            gate_s[h] = jnp.broadcast_to(gh, (8, 128))
        wr_s[...] = wr_v[...].astype(f32).reshape(1, D)

    def first_ln(s, dst, chunks=range(L // 16)):
        xsub = xb.at[pl.ds(s * L, L)]
        rsub = xres.at[pl.ds(s * L, L)]
        nsub = dst.at[pl.ds(s * (L // 2), L // 2)]
        deps = []
        for j in chunks:
            v = xsub[j * 16:(j + 1) * 16, :].astype(f32)
            rsub[j * 16:(j + 1) * 16, :] = v
            n = _pack(_ln(v))
            nsub[j * 8:(j + 1) * 8, :] = n
            deps.append(_after(pltpu.bitcast(n[:, 896:1024], f32)))
        return deps

    def out_copy(b):
        return pltpu.make_async_copy(xb.at[pl.ds(b * BR, BR)], out_hbm.at[pl.ds(b * BR, BR)], sems.at[11 + b])

    def proj_piece(src, s, w_ref, c, ties=None):
        xs = src.at[pl.ds(pl.multiple_of(s * (L // 2), L // 2), L // 2)]
        ps = [xs[:, 128 * g:128 * (g + 1)] for g in range(G)]
        for (g, v), dep in (ties or {}).items():
            ps[g] = _tie(ps[g], v, dep)
        return _dot(jnp.concatenate([_unpack(p) for p in ps], axis=1), _unpack(_wtile(w_ref, c)))

    def qkv(src, s, hooks=None):
        r0 = pl.multiple_of(s * (L // 2), L // 2)
        ties = {}
        n = 0
        for which, w_ref in ((0, wq), (1, wk), (2, wv)):
            for g in range(G):
                if hooks and n in hooks:
                    ties = hooks[n]() or ties
                y = proj_piece(src, s, w_ref, g, ties.get(n))
                if which < 2:
                    qk.at[which, g, pl.ds(r0, L // 2)][...] = _pack(((y * QSCALE) if which == 0 else y).astype(bf16))
                    pqk.at[which, g, pl.ds(r0, L // 2)][...] = _pack(_phi(y).astype(bf16))
                else:
                    vT.at[g, s][...] = _pack(y.astype(bf16).T)
                n += 1

    def step(i_qk, i_sm, Sw, Mw, Sr, Mr, filler=None, mem_read=True, mem_write=True):
        if i_qk is not None:
            gq = pl.multiple_of(i_qk % G, NI)
            rq = pl.multiple_of((i_qk // G) * (L // 2), L // 2)
            q_q = qk.at[0, pl.ds(gq, NI), pl.ds(rq, L // 2)]
            q_k = qk.at[1, pl.ds(gq, NI), pl.ds(rq, L // 2)]
        if i_sm is not None:
            gs = pl.multiple_of(i_sm % G, NI)
            ss = i_sm // G
            rs = pl.multiple_of(ss * (L // 2), L // 2)
            s_pq = pqk.at[0, pl.ds(gs, NI), pl.ds(rs, L // 2)]
            s_pk = pqk.at[1, pl.ds(gs, NI), pl.ds(rs, L // 2)]
            s_v = vT.at[pl.ds(gs, NI), ss]
            s_o = o_s.at[pl.ds(gs, NI), pl.ds(rs, L // 2)]
            s_M = Mst.at[pl.ds(gs, NI)]
            s_L = Lst.at[pl.ds(gs, NI)]
            s_g = gate_s.at[pl.ds(4 * gs, 4 * NI)]
        M, O, LS, REC, UPD = {}, {}, {}, {}, {}

        def put_scores(j, t, h, kt, sc):
            Sw.at[40 * j + TIDX[t, h, kt]][...] = sc
            mm = jnp.max(sc.reshape(16, 8, 128), axis=0)
            M[j, t, h] = jnp.maximum(M[j, t, h], mm) if (j, t, h) in M else mm

        def qk_tile(j, t, h, kt):
            kk = q_k[j, 64 * kt:64 * kt + 64, :]
            qu = q_q[j, 64 * t:64 * t + 64, :]
            if kt < t:
                put_scores(j, t, h, kt, _nt_dot(_unpack(kk & hm_s[h][0:1, :]), _unpack(qu)))
            elif h % 2 == 0:
                m0, m1 = hm_s[h][0:1, :], hm_s[h + 1][0:1, :]
                top = _nt_dot(_unpack(jnp.concatenate([kk[0:32] & m0, kk[0:32] & m1], axis=0)), _unpack(qu))
                both = jnp.concatenate([qu[32:64] & m1, qu[32:64] & m0], axis=0)
                low = _nt_dot(_unpack(kk[32:64]), _unpack(both))
                put_scores(j, t, h, kt, jnp.concatenate([top[0:64], low], axis=0) + cm_s[...])
                put_scores(j, t, h + 1, kt,
                           jnp.concatenate([top[64:128], pltpu.roll(low, 64, 1)], axis=0) + cm_s[...])
            if kt == t:
                Mw.at[16 * j + 4 * t + h][...] = jnp.broadcast_to(
                    jnp.max(M[j, t, h], axis=0, keepdims=True), (8, 128))

        def sm_tile(j, t, h, kt):
            if h == 0 and kt == 0 and mem_read:
                pq = _unpack(s_pq[j, 64 * t:64 * t + 64, :])
                REC[t] = _nt_dot(_unpack(s_L[j]), pq)
            sc = Sr[40 * j + TIDX[t, h, kt]]
            m = Mr[16 * j + 4 * t + h]
            p = jnp.exp2(sc.reshape(16, 8, 128) - m[None]).reshape(128, 128)
            ls = jnp.sum(p.reshape(16, 8, 128), axis=0)
            vt = _unpack(s_v[j, 16 * h:16 * h + 16, 128 * kt:128 * kt + 128])
            o = _dot(vt, p.astype(bf16))
            if kt == 0:
                O[t, h] = o
                LS[t, h] = ls
            else:
                O[t, h] = O[t, h] + o
                LS[t, h] = LS[t, h] + ls
            if kt == t:
                gt = s_g[4 * j + h][0:1, :]
                c2 = (1.0 - gt) * _rcp(jnp.sum(LS[t, h], axis=0, keepdims=True))
                O[t, h] = O[t, h] * c2
            if kt == t and h == 3:
                if mem_read:
                    rec = REC[t]
                    rden = _rcp(rec[128:136] + 1e-6)
                    rows = [rec[32 * hh:32 * hh + 32] * (s_g[4 * j + hh][0:1, :] * rden[hh:hh + 1, :]) + O[t, hh]
                            for hh in range(4)]
                else:
                    rows = [O[t, hh] for hh in range(4)]
                ot = jnp.concatenate(rows, axis=0).astype(bf16)
                s_o.at[j, pl.ds(64 * t, 64)][...] = _pack(ot.T)

        def mem_update_start(j):
            lhs = jnp.concatenate(
                [_unpack(s_v[j]), jnp.concatenate([_unpack(one_s[...])] * 4, axis=1)], axis=0)
            upd = _dot(lhs, _unpack(s_pk[j]))
            mn = (s_M[j] + upd[0:136]) if mem_read else upd[0:136]
            s_M.at[j][...] = mn
            hmask = jnp.concatenate([hm_s[hh] for hh in range(4) for _ in range(4)], axis=0)
            mb = pltpu.bitcast(pltpu.bitcast(mn[0:128], u32) & hmask, f32)
            sub = lax.broadcasted_iota(jnp.int32, (16, 128), 0)
            lane = lax.broadcasted_iota(jnp.int32, (16, 128), 1)
            z = jnp.broadcast_to(mn[128:129], (16, 128))
            zb = jnp.where(lane // 32 == sub, z, 0.0)
            UPD[j] = _pack(jnp.concatenate([mb, zb], axis=0).astype(bf16))

        work = [(j, x) for j in range(NI) for x in TILES]
        n_sm = 0
        for n, (j, x) in enumerate(work):
            if i_sm is not None:
                target = len(work) if i_qk is None else min(len(work), ((n + 1) * len(work)) // (len(work) - SKEW) + 1)
                target = n + 1 if i_qk is None else target
                while n_sm < target:
                    js, xs_ = work[n_sm]
                    if xs_ == TILES[0] and mem_write:
                        mem_update_start(js)
                    sm_tile(js, *xs_)
                    if xs_ == TILES[-1] and mem_write:
                        s_L.at[js][...] = UPD[js]
                    n_sm += 1
            if i_qk is not None:
                qk_tile(j, *x)
            if filler is not None:
                filler(n + 1, len(work))

    def oproj_piece(b, A, c, ties=None):
        osub = o_s.at[:, pl.ds(pl.multiple_of(b * (BR // 2), BR // 2), BR // 2)]
        ps = [osub[g] for g in range(G)]
        for (g, v), dep in (ties or {}).items():
            ps[g] = _tie(ps[g], v, dep)
        o = jnp.concatenate([_unpack(p) for p in ps], axis=1)
        A[:, 128 * c:128 * (c + 1)] = _dot(o, _unpack(_wtile(wo, c)))

    def epilogue_refs(b):
        return (xres.at[pl.ds(pl.multiple_of(b * BR, BR), BR)],
                xb.at[pl.ds(pl.multiple_of(b * BR, BR), BR)],
                xn2.at[pl.ds(pl.multiple_of(b * (BR // 2), BR // 2), BR // 2)],
                xn.at[pl.ds(pl.multiple_of(b * (BR // 2), BR // 2), BR // 2)])

    def epi1(refs, A, j, base, racc):
        xr, _, n2r, _ = refs
        rows = slice(j * 16, (j + 1) * 16)
        x1 = xr[rows, :] + A[rows, :]
        mean = jnp.mean(x1, axis=-1, keepdims=True)
        d = x1 - mean
        var = jnp.mean(d * d, axis=-1, keepdims=True)
        inv = _inv_std(var)
        n2 = d * inv
        n2r[j * 8:(j + 1) * 8, :] = _pack(n2.astype(bf16))
        r = jnp.sum(n2 * wr_s[...], axis=-1, keepdims=True)
        lane = lax.broadcasted_iota(jnp.int32, (8, 128), 1)
        racc = jnp.where(lane == base + 2 * j, r[0:8], racc)
        racc = jnp.where(lane == base + 2 * j + 1, r[8:16], racc)
        grow = 1.0 + inv
        scale2 = grow * _inv_std(var * (grow * grow))
        done = _after(jnp.broadcast_to(r[0:8] + r[8:16], (8, 128)))
        return x1, mean, d, scale2, n2, racc, done

    def epi2(refs, j, x1, d, scale2, n2, last):
        xr, xo, _, n1r = refs
        rows = slice(j * 16, (j + 1) * 16)
        x2 = x1 + n2
        xr[rows, :] = x2
        if last:
            xo[rows, :] = x2.astype(bf16)
            return _after(x2[0:8, 896:1024])
        n1 = _pack((d * scale2).astype(bf16))
        n1r[j * 8:(j + 1) * 8, :] = n1
        return _after(pltpu.bitcast(n1[:, 896:1024], f32)) | _after(x2[0:8, 896:1024])

    def put_scores(b, racc):
        half = b // 2

        @pl.when(b % 2 == 0)
        def _():
            r_s[half] = racc

        @pl.when(b % 2 == 1)
        def _():
            r_s[half] = r_s[half] + racc

    def oproj_epilogue(b, A, bn, An, last):
        refs = epilogue_refs(b)
        racc = jnp.zeros((8, 128), f32)
        deps = []
        for j in range(BR // 16):
            x1, _, d, scale2, n2, racc, done = epi1(refs, A, j, (b % 2) * (BR // 8), racc)
            deps.append(done | epi2(refs, j, x1, d, scale2, n2, last))
        ties = _spread(deps, TIE0, TIE1)
        for c in range(G):
            oproj_piece(bn, An, c, ties.get(c))
        put_scores(b, racc)

    def layer(l):
        first, last = l == 0, l == NLAYERS - 1

        with jax.named_scope("P_qkv"):
            if first:
                bufs = (xn, xn2)
                x0_copy(0).wait()
                first_ln(0, bufs[0], range(0, L // 32))
                x0_copy(1).wait()
                first_ln(0, bufs[0], range(L // 32, L // 16))
                setup_small()
                wait(wq_lo)

                def before_v0():
                    wait(wv_c)
                    x_copy(1).wait()
                    return _spread(first_ln(1, bufs[1]), 16 * 1024 + 600, 24 * 1024 - 100)

                qkv(bufs[0], 0, {2: lambda: wait(wq_mid), 5: lambda: wait(wq_hi), 8: lambda: wait(wk_c), 16: before_v0})
                for s in range(1, NSEG):
                    def before(s=s):
                        if s == 1:
                            start(wo_c)
                            start(mlp_c)
                        if s + 1 < NSEG:
                            x_copy(s + 1).wait()
                            return _spread(first_ln(s + 1, bufs[(s + 1) % 2]), 600, 16 * 1024)

                    qkv(bufs[s % 2], s, {0: before})
            else:
                lax.fori_loop(0, NSEG, lambda s, _: qkv(xn, s), None)

        nstep = 4 * G // NI
        per_seg = G // NI
        sets = ((SA, MA), (SB, MB))

        def att_step(i, **kw):
            step((i + 1) * NI, i * NI, *sets[i % 2], *sets[1 - i % 2], **kw)

        def block(fn):
            pl.when(zero_s[0] == 0)(fn)

        with jax.named_scope("P_att"):
            step(0, None, SB, MB, None, None)
            for i in range(per_seg):
                block(lambda i=i: att_step(i, mem_read=False))

            def att_body(i, _):
                @pl.when(i % 2 == 0)
                def _():
                    step((i + 1) * NI, i * NI, SA, MA, SB, MB)

                @pl.when(i % 2 == 1)
                def _():
                    step((i + 1) * NI, i * NI, SB, MB, SA, MA)

            lax.fori_loop(per_seg, nstep - per_seg, att_body, None)
            for i in range(nstep - per_seg, nstep - 1):
                block(lambda i=i: att_step(i, mem_write=False))

        if first:
            wait(wo_c)

        def filler(n, total):
            if n % (total // G) == 0:
                oproj_piece(0, AA, n // (total // G) - 1)

        with jax.named_scope("P_op"):
            if (nstep - 1) % 2 == 0:
                step(None, (nstep - 1) * NI, None, None, SB, MB, filler, mem_write=False)
            else:
                step(None, (nstep - 1) * NI, None, None, SA, MA, filler, mem_write=False)

            def op_body(i, _):
                if last:
                    @pl.when(i >= 2)
                    def _():
                        out_copy(i - 2).start()

                @pl.when(i % 2 == 1)
                def _():
                    oproj_epilogue(i - 1, AA, i, AB, last)

                @pl.when(i % 2 == 0)
                def _():
                    oproj_epilogue(i - 1, AB, i, AA, last)

            lax.fori_loop(1, NB, op_body, None)

        if last:
            out_copy(NB - 2).start()

        with jax.named_scope("P_tail"):
            with jax.named_scope("T_epi1"):
                refs = epilogue_refs(NB - 1)
                A_last = AB if (NB - 1) % 2 == 1 else AA
                racc = jnp.zeros((8, 128), f32)
                for j in range(BR // 16):
                    x1, mean, d, scale2, n2, racc, _ = epi1(refs, A_last, j, ((NB - 1) % 2) * (BR // 8), racc)
                    if last:
                        epi2(refs, j, x1, d, scale2, n2, True)
                    else:
                        A_last[j * 16:(j + 1) * 16, :] = x1
                        stat_s.at[0][j * 16:(j + 1) * 16, :] = jnp.broadcast_to(mean, (16, 128))
                        stat_s.at[1][j * 16:(j + 1) * 16, :] = jnp.broadcast_to(scale2, (16, 128))
            r_all = jnp.concatenate([r_s[0], r_s[1] + racc], axis=0)
            if last:
                out_copy(NB - 1).start()
            if first:
                wait(mlp_c)

            with jax.named_scope("T_top2"):
                rr = pltpu.bitcast(_rb(r_all), u32)
                sub = lax.broadcasted_iota(jnp.int32, (16, 128), 0)
                lane = lax.broadcasted_iota(jnp.int32, (16, 128), 1)
                pos = ((sub // 8) * 1024 + lane * 8 + (sub % 8)).astype(u32)
                neg = (rr >> 31) == 1
                key = pltpu.bitcast(rr | jnp.where(neg, pos, (S - 1) - pos), f32)

                def top(k):
                    return jnp.max(jnp.max(k, axis=1, keepdims=True), axis=0, keepdims=True)

                k1 = top(key)
                k2 = top(jnp.where(key == k1, -jnp.inf, key))

                def decode(k):
                    kb = pltpu.bitcast(jnp.broadcast_to(k, (8, 128)), u32)
                    code = kb & jnp.uint32(S - 1)
                    p = jnp.where((kb >> 31) == 1, code, (S - 1) - code).astype(jnp.int32)
                    score = pltpu.bitcast(kb & jnp.uint32(0xFFFF0000), f32)
                    return jnp.clip(jnp.max(p), 0, S - 1), score

                i1, m1 = decode(k1)
                i2, m2 = decode(k2)

            with jax.named_scope("T_pick"):
                row = lax.broadcasted_iota(jnp.int32, (16, D), 0)

                def pick(i):
                    blk = _unpack(xn2[pl.ds(pl.multiple_of((i // 16) * 8, 8), 8), :]).astype(f32)
                    return jnp.sum(jnp.where(row == i % 16, blk, 0.0), axis=0, keepdims=True)

                xs = jnp.where(row == 0, pick(i1), jnp.where(row == 1, pick(i2), 0.0)).astype(bf16)

            with jax.named_scope("T_mlp"):
                ties = {}
                if not last:
                    for j in range(BR // 16):
                        rows = slice(j * 16, (j + 1) * 16)
                        x1 = A_last[rows, :]
                        n2 = _unpack(refs[2][j * 8:(j + 1) * 8, :]).astype(f32)
                        done = epi2(refs, j, x1, x1 - stat_s[0, rows, 0:1], stat_s[1, rows, 0:1], n2, False)
                        key_ = 3 + (j * (2 * NC - 3)) // (BR // 16)
                        ties[key_] = done if key_ not in ties else ties[key_] | done

                def weights(w_ref, c, key_):
                    tiles = [_wtile(w_ref, 4 * c + t) for t in range(4)] if key_ in ties else None
                    if tiles is None:
                        return _cols(w_ref, 4 * c, 4)
                    tiles[0] = _tie(tiles[0], 0, ties[key_])
                    return jnp.concatenate([_unpack(t) for t in tiles], axis=1)

                def gate_up(c):
                    gg = _rb(_dot(xs, weights(wg, c, 2 * c)))
                    uu = _rb(_dot(xs, weights(wu, c, 2 * c + 1)))
                    return (_rb(gg * jax.nn.sigmoid(gg)) * uu).astype(bf16)

                y = jnp.zeros((16, D), f32)
                a = gate_up(0)
                for c in range(NC):
                    a_next = gate_up(c + 1) if c + 1 < NC else None
                    y = y + _dot(a, _cols(wd, 0, G, c * FC, FC))
                    a = a_next
                row8 = lax.broadcasted_iota(jnp.int32, (16, 128), 0)
                gsel = _rb(jax.nn.sigmoid(jnp.where(row8 == 0, m1[0:1, :], m2[0:1, :])))
                upd = _rb(_rb(y) * jnp.concatenate([gsel] * (D // 128), axis=1))

            with jax.named_scope("T_fix"):
                def rows_at(i):
                    return pl.multiple_of((i // 16) * 16, 16)

                def updated(i0):
                    xv = xres[pl.ds(rows_at(i0), 16), :]
                    for i, j in ((i1, 0), (i2, 1)):
                        hit = (row == i % 16) & (i // 16 == i0 // 16)
                        xv = xv + jnp.where(hit, upd[j:j + 1, :], 0.0)
                    return xv.astype(bf16)

                xv1, xv2 = updated(i1), updated(i2)
                if last:
                    patch[0] = xv1
                    patch[1] = xv2
                    for b in range(NB):
                        out_copy(b).wait()
                    b1, b2 = rows_at(i1), rows_at(i2)
                    c1 = pltpu.make_async_copy(patch.at[0], out_hbm.at[pl.ds(b1, 16)], sems.at[15])
                    c2 = pltpu.make_async_copy(patch.at[1], out_hbm.at[pl.ds(b2, 16)], sems.at[16])

                    @pl.when(b1 != b2)
                    def _():
                        c1.start()

                    c2.start()

                    @pl.when(b1 != b2)
                    def _():
                        c1.wait()

                    c2.wait()
                else:
                    n1, n2 = _pack(_ln(xv1.astype(f32))), _pack(_ln(xv2.astype(f32)))
                    for i, xv, nn in ((i1, xv1, n1), (i2, xv2, n2)):
                        xres[pl.ds(rows_at(i), 16), :] = xv.astype(f32)
                        xn.at[pl.ds(pl.multiple_of((i // 16) * 8, 8), 8)][...] = nn

    for l in range(NLAYERS):
        layer(l)


@jax.jit
def pallas_interleave_layers__memory_aug_infini_attn__moe_arch_mod__prompt_kernel(
    A_x, A_wq, A_wk, A_wv, A_wo, A_beta, B_x, B_w_r, B_w_gate, B_w_up, B_w_down,
):
    del B_x
    x = A_x.reshape(S, D)
    hbm = pl.BlockSpec(memory_space=pltpu.HBM)
    scratch = [
        pltpu.VMEM((S, D), bf16),
        pltpu.VMEM((D // 128, D, 128), bf16),
        pltpu.VMEM((D // 128, D, 128), bf16),
        pltpu.VMEM((D // 128, D, 128), bf16),
        pltpu.VMEM((D // 128, D, 128), bf16),
        pltpu.VMEM((F // 128, D, 128), bf16),
        pltpu.VMEM((F // 128, D, 128), bf16),
        pltpu.VMEM((D // 128, F, 128), bf16),
        pltpu.VMEM((H,), bf16),
        pltpu.VMEM((D,), bf16),
        pltpu.VMEM((S, D), f32),
        pltpu.VMEM((S // 2, D), u32),
        pltpu.VMEM((2, G, S // 2, 128), u32),
        pltpu.VMEM((2, G, S // 2, 128), u32),
        pltpu.VMEM((G, NSEG, 64, L), u32),
        pltpu.VMEM((G, S // 2, 128), u32),
        pltpu.VMEM((40 * NI, 128, 128), f32),
        pltpu.VMEM((40 * NI, 128, 128), f32),
        pltpu.VMEM((16 * NI, 8, 128), f32),
        pltpu.VMEM((16 * NI, 8, 128), f32),
        pltpu.VMEM((G, 136, 128), f32),
        pltpu.VMEM((G, 72, 128), u32),
        pltpu.VMEM((BR, D), f32),
        pltpu.VMEM((BR, D), f32),
        pltpu.VMEM((S // 2, D), u32),
        pltpu.VMEM((2, 8, 128), f32),
        pltpu.VMEM((4, 8, 128), u32),
        pltpu.VMEM((128, 128), f32),
        pltpu.VMEM((H, 8, 128), f32),
        pltpu.VMEM((8, 128), u32),
        pltpu.VMEM((2, 16, D), bf16),
        pltpu.VMEM((2, BR, 128), f32),
        pltpu.VMEM((1, D), f32),
        pltpu.SMEM((1,), jnp.int32),
        pltpu.SemaphoreType.DMA((20,)),
    ]
    out = pl.pallas_call(
        _kernel,
        out_shape=jax.ShapeDtypeStruct((S, D), bf16),
        in_specs=[hbm] * 10,
        out_specs=hbm,
        scratch_shapes=scratch,
        compiler_params=pltpu.CompilerParams(vmem_limit_bytes=124 * 1024 * 1024),
        name="infini_mod_kernel",
    )(x, A_wq, A_wk, A_wv, A_wo, A_beta, B_w_r, B_w_gate, B_w_up, B_w_down)
    return out.reshape(1, S, D)
```

```python
import math

import jax
import jax.numpy as jnp
from jax import lax
import jax.experimental.pallas as pl
import jax.experimental.pallas.tpu as pltpu

S = 2048
D = 1024
H = 32
DH = 32
NSEG = 4
L = S // NSEG
G = 8
F = 3584
BR = 512
NB = S // BR
NI = 4
SKEW = 8
TIE0, TIE1 = 600, 8150
FC = 512
NC = F // FC
NLAYERS = 2

f32 = jnp.float32
bf16 = jnp.bfloat16
u32 = jnp.uint32

EPS_B = 1.0013580322265625e-05
SCALE_B = 0.1767578125
LOG2E = math.log2(math.e)
QSCALE = SCALE_B * LOG2E
NEG = -1e30

TILES = [(t, h, kt) for t in range(4) for h in range(4) for kt in range(t + 1)]
TIDX = {x: i for i, x in enumerate(TILES)}


def _rb(v):
    return v.astype(bf16).astype(f32)


def _pack(v):
    return pltpu.bitcast(v, u32)


def _unpack(v):
    return pltpu.bitcast(v, bf16)


def _rcp(v):
    y = pltpu.reciprocal(v, approx=True)
    return y * (2.0 - v * y)


def _inv_std(var):
    return _rcp(_rb(jnp.exp2(0.5 * jnp.log2(_rb(_rb(var) + EPS_B)))))


def _rsqrt_eps(var):
    return jnp.exp2(-0.5 * jnp.log2(var + EPS_B))


def _ln(v):
    d = v - jnp.mean(v, axis=-1, keepdims=True)
    return (d * _rsqrt_eps(jnp.mean(d * d, axis=-1, keepdims=True))).astype(bf16)


def _after(v):
    return jnp.where(v != v, jnp.uint32(1), jnp.uint32(0)) & jnp.uint32(0x10)


def _tie(p, v, dep):
    parts = [p[:8 * v]] if v else []
    parts.append(p[8 * v:8 * v + 8] | dep)
    if 8 * v + 8 < p.shape[0]:
        parts.append(p[8 * v + 8:])
    return jnp.concatenate(parts, axis=0) if len(parts) > 1 else parts[0]


def _phi(t):
    return jnp.where(t > 0, t + 1.0, jnp.exp(t))


def _nt_dot(a, b):
    return lax.dot_general(a, b, (((1,), (1,)), ((), ())), preferred_element_type=f32)


def _dot(a, b):
    return jnp.dot(a, b, preferred_element_type=f32)


def _wtile(ref, c, r0=0, nr=None):
    nr = ref.shape[1] if nr is None else nr
    return ref.bitcast(u32)[c, r0 // 2:(r0 + nr) // 2, :]


def _cols(ref, c0, n, r0=0, nr=None):
    return jnp.concatenate([_unpack(_wtile(ref, c, r0, nr)) for c in range(c0, c0 + n)], axis=1)


def _spread(deps, t0, t1):
    ties = {}
    for j, dep in enumerate(deps):
        when = t0 + (j * (t1 - t0)) // (len(deps) - 1)
        slot = ties.setdefault(when // 1024, {})
        key = (4 * ((when % 1024) // 512), (when % 512) // 16)
        slot[key] = dep if key not in slot else slot[key] | dep
    return ties


def _kernel(x_hbm, wq_hbm, wk_hbm, wv_hbm, wo_hbm, beta_hbm, wr_hbm, wg_hbm, wu_hbm, wd_hbm,
            out_hbm,
            xb, wq, wk, wv, wo, wg, wu, wd, beta_v, wr_v,
            xres, xn, qk, pqk, vT, o_s, SA, SB, MA, MB, Mst, Lst, AA, AB, xn2, r_s,
            hm_s, cm_s, gate_s, one_s, patch, stat_s, wr_s, zero_s, sems):
    def x_copy(s):
        r = pl.ds(pl.multiple_of(s * L, L), L)
        return pltpu.make_async_copy(x_hbm.at[r], xb.at[r], sems.at[s])

    def w_copies(src, dst, sem, c0=0, c1=None):
        c1 = dst.shape[0] if c1 is None else c1
        return [pltpu.make_async_copy(src.at[:, pl.ds(128 * c, 128)], dst.at[c], sems.at[sem])
                for c in range(c0, c1)]

    def start(copies):
        for c in copies:
            c.start()

    def wait(copies):
        for c in copies:
            c.wait()

    beta_c = pltpu.make_async_copy(beta_hbm, beta_v, sems.at[4])
    wr_c = pltpu.make_async_copy(wr_hbm, wr_v, sems.at[4])
    wq_lo, wq_mid, wq_hi = w_copies(wq_hbm, wq, 5, 0, 2), w_copies(wq_hbm, wq, 19, 2, 5), w_copies(wq_hbm, wq, 6, 5, 8)
    wk_c, wv_c, wo_c = w_copies(wk_hbm, wk, 7), w_copies(wv_hbm, wv, 8), w_copies(wo_hbm, wo, 9)
    mlp_c = w_copies(wg_hbm, wg, 10) + w_copies(wu_hbm, wu, 10) + w_copies(wd_hbm, wd, 10)

    def x0_copy(h):
        r = pl.ds(h * (L // 2), L // 2)
        return pltpu.make_async_copy(x_hbm.at[r], xb.at[r], sems.at[17 + h])

    beta_c.start()
    wr_c.start()
    x0_copy(0).start()
    x0_copy(1).start()
    start(wq_lo)
    start(wq_mid)
    start(wq_hi)
    start(wk_c)
    x_copy(1).start()
    start(wv_c)
    x_copy(2).start()
    x_copy(3).start()

    zero_s[0] = 0
    lane8 = lax.broadcasted_iota(jnp.int32, (8, 128), 1)
    for h in range(4):
        hm_s[h] = jnp.where((lane8 >= 32 * h) & (lane8 < 32 * h + 32), jnp.uint32(0xFFFFFFFF), jnp.uint32(0))
    ki = lax.broadcasted_iota(jnp.int32, (128, 128), 0)
    qi = lax.broadcasted_iota(jnp.int32, (128, 128), 1)
    cm_s[...] = jnp.where(ki <= qi, 0.0, NEG).astype(f32)
    row16 = lax.broadcasted_iota(jnp.int32, (16, 128), 0)
    one_s[...] = _pack(jnp.where(row16 == 0, 1.0, 0.0).astype(bf16))

    def setup_small():
        beta_c.wait()
        wr_c.wait()
        gate_row = jnp.broadcast_to(jax.nn.sigmoid(beta_v[...].astype(f32).reshape(1, H)), (8, H))
        lane_h = lax.broadcasted_iota(jnp.int32, (8, H), 1)
        for h in range(H):
            gh = jnp.sum(jnp.where(lane_h == h, gate_row, 0.0), axis=-1, keepdims=True)
            gate_s[h] = jnp.broadcast_to(gh, (8, 128))
        wr_s[...] = wr_v[...].astype(f32).reshape(1, D)

    def first_ln(s, dst, chunks=range(L // 16)):
        xsub = xb.at[pl.ds(s * L, L)]
        rsub = xres.at[pl.ds(s * L, L)]
        nsub = dst.at[pl.ds(s * (L // 2), L // 2)]
        deps = []
        for j in chunks:
            v = xsub[j * 16:(j + 1) * 16, :].astype(f32)
            rsub[j * 16:(j + 1) * 16, :] = v
            n = _pack(_ln(v))
            nsub[j * 8:(j + 1) * 8, :] = n
            deps.append(_after(pltpu.bitcast(n[:, 896:1024], f32)))
        return deps

    def out_copy(b):
        return pltpu.make_async_copy(xb.at[pl.ds(b * BR, BR)], out_hbm.at[pl.ds(b * BR, BR)], sems.at[11 + b])

    def proj_piece(src, s, w_ref, c, ties=None):
        xs = src.at[pl.ds(pl.multiple_of(s * (L // 2), L // 2), L // 2)]
        ps = [xs[:, 128 * g:128 * (g + 1)] for g in range(G)]
        for (g, v), dep in (ties or {}).items():
            ps[g] = _tie(ps[g], v, dep)
        return _dot(jnp.concatenate([_unpack(p) for p in ps], axis=1), _unpack(_wtile(w_ref, c)))

    def qkv(src, s, hooks=None):
        r0 = pl.multiple_of(s * (L // 2), L // 2)
        ties = {}
        n = 0
        for which, w_ref in ((0, wq), (1, wk), (2, wv)):
            for g in range(G):
                if hooks and n in hooks:
                    ties = hooks[n]() or ties
                y = proj_piece(src, s, w_ref, g, ties.get(n))
                if which < 2:
                    qk.at[which, g, pl.ds(r0, L // 2)][...] = _pack(((y * QSCALE) if which == 0 else y).astype(bf16))
                    pqk.at[which, g, pl.ds(r0, L // 2)][...] = _pack(_phi(y).astype(bf16))
                else:
                    vT.at[g, s][...] = _pack(y.astype(bf16).T)
                n += 1

    def step(i_qk, i_sm, Sw, Mw, Sr, Mr, filler=None, mem_read=True, mem_write=True):
        if i_qk is not None:
            gq = pl.multiple_of(i_qk % G, NI)
            rq = pl.multiple_of((i_qk // G) * (L // 2), L // 2)
            q_q = qk.at[0, pl.ds(gq, NI), pl.ds(rq, L // 2)]
            q_k = qk.at[1, pl.ds(gq, NI), pl.ds(rq, L // 2)]
        if i_sm is not None:
            gs = pl.multiple_of(i_sm % G, NI)
            ss = i_sm // G
            rs = pl.multiple_of(ss * (L // 2), L // 2)
            s_pq = pqk.at[0, pl.ds(gs, NI), pl.ds(rs, L // 2)]
            s_pk = pqk.at[1, pl.ds(gs, NI), pl.ds(rs, L // 2)]
            s_v = vT.at[pl.ds(gs, NI), ss]
            s_o = o_s.at[pl.ds(gs, NI), pl.ds(rs, L // 2)]
            s_M = Mst.at[pl.ds(gs, NI)]
            s_L = Lst.at[pl.ds(gs, NI)]
            s_g = gate_s.at[pl.ds(4 * gs, 4 * NI)]
        M, O, LS, REC, UPD = {}, {}, {}, {}, {}

        def put_scores(j, t, h, kt, sc):
            Sw.at[40 * j + TIDX[t, h, kt]][...] = sc
            mm = jnp.max(sc.reshape(16, 8, 128), axis=0)
            M[j, t, h] = jnp.maximum(M[j, t, h], mm) if (j, t, h) in M else mm

        def qk_tile(j, t, h, kt):
            kk = q_k[j, 64 * kt:64 * kt + 64, :]
            qu = q_q[j, 64 * t:64 * t + 64, :]
            if kt < t:
                put_scores(j, t, h, kt, _nt_dot(_unpack(kk & hm_s[h][0:1, :]), _unpack(qu)))
            elif h % 2 == 0:
                m0, m1 = hm_s[h][0:1, :], hm_s[h + 1][0:1, :]
                top = _nt_dot(_unpack(jnp.concatenate([kk[0:32] & m0, kk[0:32] & m1], axis=0)), _unpack(qu))
                both = jnp.concatenate([qu[32:64] & m1, qu[32:64] & m0], axis=0)
                low = _nt_dot(_unpack(kk[32:64]), _unpack(both))
                put_scores(j, t, h, kt, jnp.concatenate([top[0:64], low], axis=0) + cm_s[...])
                put_scores(j, t, h + 1, kt,
                           jnp.concatenate([top[64:128], pltpu.roll(low, 64, 1)], axis=0) + cm_s[...])
            if kt == t:
                Mw.at[16 * j + 4 * t + h][...] = jnp.broadcast_to(
                    jnp.max(M[j, t, h], axis=0, keepdims=True), (8, 128))

        def sm_tile(j, t, h, kt):
            if h == 0 and kt == 0 and mem_read:
                pq = _unpack(s_pq[j, 64 * t:64 * t + 64, :])
                REC[t] = _nt_dot(_unpack(s_L[j]), pq)
            sc = Sr[40 * j + TIDX[t, h, kt]]
            m = Mr[16 * j + 4 * t + h]
            p = jnp.exp2(sc.reshape(16, 8, 128) - m[None]).reshape(128, 128)
            ls = jnp.sum(p.reshape(16, 8, 128), axis=0)
            vt = _unpack(s_v[j, 16 * h:16 * h + 16, 128 * kt:128 * kt + 128])
            o = _dot(vt, p.astype(bf16))
            if kt == 0:
                O[t, h] = o
                LS[t, h] = ls
            else:
                O[t, h] = O[t, h] + o
                LS[t, h] = LS[t, h] + ls
            if kt == t:
                gt = s_g[4 * j + h][0:1, :]
                c2 = (1.0 - gt) * _rcp(jnp.sum(LS[t, h], axis=0, keepdims=True))
                O[t, h] = O[t, h] * c2
            if kt == t and h == 3:
                if mem_read:
                    rec = REC[t]
                    rden = _rcp(rec[128:136] + 1e-6)
                    rows = [rec[32 * hh:32 * hh + 32] * (s_g[4 * j + hh][0:1, :] * rden[hh:hh + 1, :]) + O[t, hh]
                            for hh in range(4)]
                else:
                    rows = [O[t, hh] for hh in range(4)]
                ot = jnp.concatenate(rows, axis=0).astype(bf16)
                s_o.at[j, pl.ds(64 * t, 64)][...] = _pack(ot.T)

        def mem_update_start(j):
            lhs = jnp.concatenate(
                [_unpack(s_v[j]), jnp.concatenate([_unpack(one_s[...])] * 4, axis=1)], axis=0)
            upd = _dot(lhs, _unpack(s_pk[j]))
            mn = (s_M[j] + upd[0:136]) if mem_read else upd[0:136]
            s_M.at[j][...] = mn
            hmask = jnp.concatenate([hm_s[hh] for hh in range(4) for _ in range(4)], axis=0)
            mb = pltpu.bitcast(pltpu.bitcast(mn[0:128], u32) & hmask, f32)
            sub = lax.broadcasted_iota(jnp.int32, (16, 128), 0)
            lane = lax.broadcasted_iota(jnp.int32, (16, 128), 1)
            z = jnp.broadcast_to(mn[128:129], (16, 128))
            zb = jnp.where(lane // 32 == sub, z, 0.0)
            UPD[j] = _pack(jnp.concatenate([mb, zb], axis=0).astype(bf16))

        work = [(j, x) for j in range(NI) for x in TILES]
        n_sm = 0
        for n, (j, x) in enumerate(work):
            if i_sm is not None:
                target = len(work) if i_qk is None else min(len(work), ((n + 1) * len(work)) // (len(work) - SKEW) + 1)
                target = n + 1 if i_qk is None else target
                while n_sm < target:
                    js, xs_ = work[n_sm]
                    if xs_ == TILES[0] and mem_write:
                        mem_update_start(js)
                    sm_tile(js, *xs_)
                    if xs_ == TILES[-1] and mem_write:
                        s_L.at[js][...] = UPD[js]
                    n_sm += 1
            if i_qk is not None:
                qk_tile(j, *x)
            if filler is not None:
                filler(n + 1, len(work))

    def oproj_piece(b, A, c, ties=None):
        osub = o_s.at[:, pl.ds(pl.multiple_of(b * (BR // 2), BR // 2), BR // 2)]
        ps = [osub[g] for g in range(G)]
        for (g, v), dep in (ties or {}).items():
            ps[g] = _tie(ps[g], v, dep)
        o = jnp.concatenate([_unpack(p) for p in ps], axis=1)
        A[:, 128 * c:128 * (c + 1)] = _dot(o, _unpack(_wtile(wo, c)))

    def epilogue_refs(b):
        return (xres.at[pl.ds(pl.multiple_of(b * BR, BR), BR)],
                xb.at[pl.ds(pl.multiple_of(b * BR, BR), BR)],
                xn2.at[pl.ds(pl.multiple_of(b * (BR // 2), BR // 2), BR // 2)],
                xn.at[pl.ds(pl.multiple_of(b * (BR // 2), BR // 2), BR // 2)])

    def epi1(refs, A, j, base, racc):
        xr, _, n2r, _ = refs
        rows = slice(j * 16, (j + 1) * 16)
        x1 = xr[rows, :] + A[rows, :]
        mean = jnp.mean(x1, axis=-1, keepdims=True)
        d = x1 - mean
        var = jnp.mean(d * d, axis=-1, keepdims=True)
        inv = _inv_std(var)
        n2 = d * inv
        n2r[j * 8:(j + 1) * 8, :] = _pack(n2.astype(bf16))
        r = jnp.sum(n2 * wr_s[...], axis=-1, keepdims=True)
        lane = lax.broadcasted_iota(jnp.int32, (8, 128), 1)
        racc = jnp.where(lane == base + 2 * j, r[0:8], racc)
        racc = jnp.where(lane == base + 2 * j + 1, r[8:16], racc)
        grow = 1.0 + inv
        scale2 = grow * _rsqrt_eps(var * (grow * grow))
        done = _after(jnp.broadcast_to(r[0:8] + r[8:16], (8, 128)))
        return x1, mean, d, scale2, n2, racc, done

    def epi2(refs, j, x1, d, scale2, n2, last):
        xr, xo, _, n1r = refs
        rows = slice(j * 16, (j + 1) * 16)
        x2 = x1 + n2
        xr[rows, :] = x2
        if last:
            xo[rows, :] = x2.astype(bf16)
            return _after(x2[0:8, 896:1024])
        n1 = _pack((d * scale2).astype(bf16))
        n1r[j * 8:(j + 1) * 8, :] = n1
        return _after(pltpu.bitcast(n1[:, 896:1024], f32)) | _after(x2[0:8, 896:1024])

    def put_scores(b, racc):
        half = b // 2

        @pl.when(b % 2 == 0)
        def _():
            r_s[half] = racc

        @pl.when(b % 2 == 1)
        def _():
            r_s[half] = r_s[half] + racc

    def oproj_epilogue(b, A, bn, An, last):
        refs = epilogue_refs(b)
        racc = jnp.zeros((8, 128), f32)
        deps = []
        for j in range(BR // 16):
            x1, _, d, scale2, n2, racc, done = epi1(refs, A, j, (b % 2) * (BR // 8), racc)
            deps.append(done | epi2(refs, j, x1, d, scale2, n2, last))
        ties = _spread(deps, TIE0, TIE1)
        for c in range(G):
            oproj_piece(bn, An, c, ties.get(c))
        put_scores(b, racc)

    def layer(l):
        first, last = l == 0, l == NLAYERS - 1

        with jax.named_scope("P_qkv"):
            if first:
                bufs = (xn, xn2)
                x0_copy(0).wait()
                first_ln(0, bufs[0], range(0, L // 32))
                x0_copy(1).wait()
                first_ln(0, bufs[0], range(L // 32, L // 16))
                setup_small()
                wait(wq_lo)

                def before_v0():
                    wait(wv_c)
                    x_copy(1).wait()
                    return _spread(first_ln(1, bufs[1]), 16 * 1024 + 600, 24 * 1024 - 100)

                qkv(bufs[0], 0, {2: lambda: wait(wq_mid), 5: lambda: wait(wq_hi), 8: lambda: wait(wk_c), 16: before_v0})
                for s in range(1, NSEG):
                    def before(s=s):
                        if s == 1:
                            start(wo_c)
                            start(mlp_c)
                        if s + 1 < NSEG:
                            x_copy(s + 1).wait()
                            return _spread(first_ln(s + 1, bufs[(s + 1) % 2]), 600, 16 * 1024)

                    qkv(bufs[s % 2], s, {0: before})
            else:
                lax.fori_loop(0, NSEG, lambda s, _: qkv(xn, s), None)

        nstep = 4 * G // NI
        per_seg = G // NI
        sets = ((SA, MA), (SB, MB))

        def att_step(i, **kw):
            step((i + 1) * NI, i * NI, *sets[i % 2], *sets[1 - i % 2], **kw)

        def block(fn):
            pl.when(zero_s[0] == 0)(fn)

        with jax.named_scope("P_att"):
            step(0, None, SB, MB, None, None)
            for i in range(per_seg):
                block(lambda i=i: att_step(i, mem_read=False))

            def att_body(i, _):
                @pl.when(i % 2 == 0)
                def _():
                    step((i + 1) * NI, i * NI, SA, MA, SB, MB)

                @pl.when(i % 2 == 1)
                def _():
                    step((i + 1) * NI, i * NI, SB, MB, SA, MA)

            lax.fori_loop(per_seg, nstep - per_seg, att_body, None)
            for i in range(nstep - per_seg, nstep - 1):
                block(lambda i=i: att_step(i, mem_write=False))

        if first:
            wait(wo_c)

        def filler(n, total):
            if n % (total // G) == 0:
                oproj_piece(0, AA, n // (total // G) - 1)

        with jax.named_scope("P_op"):
            if (nstep - 1) % 2 == 0:
                step(None, (nstep - 1) * NI, None, None, SB, MB, filler, mem_write=False)
            else:
                step(None, (nstep - 1) * NI, None, None, SA, MA, filler, mem_write=False)

            def op_body(i, _):
                if last:
                    @pl.when(i >= 2)
                    def _():
                        out_copy(i - 2).start()

                @pl.when(i % 2 == 1)
                def _():
                    oproj_epilogue(i - 1, AA, i, AB, last)

                @pl.when(i % 2 == 0)
                def _():
                    oproj_epilogue(i - 1, AB, i, AA, last)

            lax.fori_loop(1, NB, op_body, None)

        if last:
            out_copy(NB - 2).start()

        with jax.named_scope("P_tail"):
            with jax.named_scope("T_epi1"):
                refs = epilogue_refs(NB - 1)
                A_last = AB if (NB - 1) % 2 == 1 else AA
                racc = jnp.zeros((8, 128), f32)
                for j in range(BR // 16):
                    x1, mean, d, scale2, n2, racc, _ = epi1(refs, A_last, j, ((NB - 1) % 2) * (BR // 8), racc)
                    if last:
                        epi2(refs, j, x1, d, scale2, n2, True)
                    else:
                        A_last[j * 16:(j + 1) * 16, :] = x1
                        stat_s.at[0][j * 16:(j + 1) * 16, :] = jnp.broadcast_to(mean, (16, 128))
                        stat_s.at[1][j * 16:(j + 1) * 16, :] = jnp.broadcast_to(scale2, (16, 128))
            r_all = jnp.concatenate([r_s[0], r_s[1] + racc], axis=0)
            if last:
                out_copy(NB - 1).start()
            if first:
                wait(mlp_c)

            with jax.named_scope("T_top2"):
                rr = pltpu.bitcast(_rb(r_all), u32)
                sub = lax.broadcasted_iota(jnp.int32, (16, 128), 0)
                lane = lax.broadcasted_iota(jnp.int32, (16, 128), 1)
                pos = ((sub // 8) * 1024 + lane * 8 + (sub % 8)).astype(u32)
                neg = (rr >> 31) == 1
                key = pltpu.bitcast(rr | jnp.where(neg, pos, (S - 1) - pos), f32)

                def top(k):
                    return jnp.max(jnp.max(k, axis=1, keepdims=True), axis=0, keepdims=True)

                k1 = top(key)
                k2 = top(jnp.where(key == k1, -jnp.inf, key))

                def decode(k):
                    kb = pltpu.bitcast(jnp.broadcast_to(k, (8, 128)), u32)
                    code = kb & jnp.uint32(S - 1)
                    p = jnp.where((kb >> 31) == 1, code, (S - 1) - code).astype(jnp.int32)
                    score = pltpu.bitcast(kb & jnp.uint32(0xFFFF0000), f32)
                    return jnp.clip(jnp.max(p), 0, S - 1), score

                i1, m1 = decode(k1)
                i2, m2 = decode(k2)

            with jax.named_scope("T_pick"):
                row = lax.broadcasted_iota(jnp.int32, (16, D), 0)

                def pick(i):
                    blk = _unpack(xn2[pl.ds(pl.multiple_of((i // 16) * 8, 8), 8), :]).astype(f32)
                    return jnp.sum(jnp.where(row == i % 16, blk, 0.0), axis=0, keepdims=True)

                xs = jnp.where(row == 0, pick(i1), jnp.where(row == 1, pick(i2), 0.0)).astype(bf16)

            with jax.named_scope("T_mlp"):
                ties = {}
                if not last:
                    for j in range(BR // 16):
                        rows = slice(j * 16, (j + 1) * 16)
                        x1 = A_last[rows, :]
                        n2 = _unpack(refs[2][j * 8:(j + 1) * 8, :]).astype(f32)
                        done = epi2(refs, j, x1, x1 - stat_s[0, rows, 0:1], stat_s[1, rows, 0:1], n2, False)
                        key_ = 3 + (j * (2 * NC - 3)) // (BR // 16)
                        ties[key_] = done if key_ not in ties else ties[key_] | done

                def weights(w_ref, c, key_):
                    tiles = [_wtile(w_ref, 4 * c + t) for t in range(4)] if key_ in ties else None
                    if tiles is None:
                        return _cols(w_ref, 4 * c, 4)
                    tiles[0] = _tie(tiles[0], 0, ties[key_])
                    return jnp.concatenate([_unpack(t) for t in tiles], axis=1)

                def gate_up(c):
                    gg = _rb(_dot(xs, weights(wg, c, 2 * c)))
                    uu = _rb(_dot(xs, weights(wu, c, 2 * c + 1)))
                    return (_rb(gg * jax.nn.sigmoid(gg)) * uu).astype(bf16)

                y = jnp.zeros((16, D), f32)
                a = gate_up(0)
                for c in range(NC):
                    a_next = gate_up(c + 1) if c + 1 < NC else None
                    y = y + _dot(a, _cols(wd, 0, G, c * FC, FC))
                    a = a_next
                row8 = lax.broadcasted_iota(jnp.int32, (16, 128), 0)
                gsel = _rb(jax.nn.sigmoid(jnp.where(row8 == 0, m1[0:1, :], m2[0:1, :])))
                upd = _rb(_rb(y) * jnp.concatenate([gsel] * (D // 128), axis=1))

            with jax.named_scope("T_fix"):
                def rows_at(i):
                    return pl.multiple_of((i // 16) * 16, 16)

                def updated(i0):
                    xv = xres[pl.ds(rows_at(i0), 16), :]
                    for i, j in ((i1, 0), (i2, 1)):
                        hit = (row == i % 16) & (i // 16 == i0 // 16)
                        xv = xv + jnp.where(hit, upd[j:j + 1, :], 0.0)
                    return xv.astype(bf16)

                xv1, xv2 = updated(i1), updated(i2)
                if last:
                    patch[0] = xv1
                    patch[1] = xv2
                    for b in range(NB):
                        out_copy(b).wait()
                    b1, b2 = rows_at(i1), rows_at(i2)
                    c1 = pltpu.make_async_copy(patch.at[0], out_hbm.at[pl.ds(b1, 16)], sems.at[15])
                    c2 = pltpu.make_async_copy(patch.at[1], out_hbm.at[pl.ds(b2, 16)], sems.at[16])

                    @pl.when(b1 != b2)
                    def _():
                        c1.start()

                    c2.start()

                    @pl.when(b1 != b2)
                    def _():
                        c1.wait()

                    c2.wait()
                else:
                    n1, n2 = _pack(_ln(xv1.astype(f32))), _pack(_ln(xv2.astype(f32)))
                    for i, xv, nn in ((i1, xv1, n1), (i2, xv2, n2)):
                        xres[pl.ds(rows_at(i), 16), :] = xv.astype(f32)
                        xn.at[pl.ds(pl.multiple_of((i // 16) * 8, 8), 8)][...] = nn

    for l in range(NLAYERS):
        layer(l)


@jax.jit
def pallas_interleave_layers__memory_aug_infini_attn__moe_arch_mod__prompt_kernel(
    A_x, A_wq, A_wk, A_wv, A_wo, A_beta, B_x, B_w_r, B_w_gate, B_w_up, B_w_down,
):
    del B_x
    x = A_x.reshape(S, D)
    hbm = pl.BlockSpec(memory_space=pltpu.HBM)
    scratch = [
        pltpu.VMEM((S, D), bf16),
        pltpu.VMEM((D // 128, D, 128), bf16),
        pltpu.VMEM((D // 128, D, 128), bf16),
        pltpu.VMEM((D // 128, D, 128), bf16),
        pltpu.VMEM((D // 128, D, 128), bf16),
        pltpu.VMEM((F // 128, D, 128), bf16),
        pltpu.VMEM((F // 128, D, 128), bf16),
        pltpu.VMEM((D // 128, F, 128), bf16),
        pltpu.VMEM((H,), bf16),
        pltpu.VMEM((D,), bf16),
        pltpu.VMEM((S, D), f32),
        pltpu.VMEM((S // 2, D), u32),
        pltpu.VMEM((2, G, S // 2, 128), u32),
        pltpu.VMEM((2, G, S // 2, 128), u32),
        pltpu.VMEM((G, NSEG, 64, L), u32),
        pltpu.VMEM((G, S // 2, 128), u32),
        pltpu.VMEM((40 * NI, 128, 128), f32),
        pltpu.VMEM((40 * NI, 128, 128), f32),
        pltpu.VMEM((16 * NI, 8, 128), f32),
        pltpu.VMEM((16 * NI, 8, 128), f32),
        pltpu.VMEM((G, 136, 128), f32),
        pltpu.VMEM((G, 72, 128), u32),
        pltpu.VMEM((BR, D), f32),
        pltpu.VMEM((BR, D), f32),
        pltpu.VMEM((S // 2, D), u32),
        pltpu.VMEM((2, 8, 128), f32),
        pltpu.VMEM((4, 8, 128), u32),
        pltpu.VMEM((128, 128), f32),
        pltpu.VMEM((H, 8, 128), f32),
        pltpu.VMEM((8, 128), u32),
        pltpu.VMEM((2, 16, D), bf16),
        pltpu.VMEM((2, BR, 128), f32),
        pltpu.VMEM((1, D), f32),
        pltpu.SMEM((1,), jnp.int32),
        pltpu.SemaphoreType.DMA((20,)),
    ]
    out = pl.pallas_call(
        _kernel,
        out_shape=jax.ShapeDtypeStruct((S, D), bf16),
        in_specs=[hbm] * 10,
        out_specs=hbm,
        scratch_shapes=scratch,
        compiler_params=pltpu.CompilerParams(vmem_limit_bytes=124 * 1024 * 1024),
        name="infini_mod_kernel",
    )(x, A_wq, A_wk, A_wv, A_wo, A_beta, B_w_r, B_w_gate, B_w_up, B_w_down)
    return out.reshape(1, S, D)
```

```python
import math

import jax
import jax.numpy as jnp
from jax import lax
import jax.experimental.pallas as pl
import jax.experimental.pallas.tpu as pltpu

S = 2048
D = 1024
H = 32
DH = 32
NSEG = 4
L = S // NSEG
G = 8
F = 3584
BR = 512
NB = S // BR
NI = 4
SKEW = 8
TIE0, TIE1 = 600, 8150
FC = 512
NC = F // FC
NLAYERS = 2

f32 = jnp.float32
bf16 = jnp.bfloat16
u32 = jnp.uint32

EPS_B = 1.0013580322265625e-05
SCALE_B = 0.1767578125
LOG2E = math.log2(math.e)
QSCALE = SCALE_B * LOG2E
NEG = -1e30

TILES = [(t, h, kt) for t in range(4) for h in range(4) for kt in range(t + 1)]
TIDX = {x: i for i, x in enumerate(TILES)}


def _rb(v):
    return v.astype(bf16).astype(f32)


def _pack(v):
    return pltpu.bitcast(v, u32)


def _unpack(v):
    return pltpu.bitcast(v, bf16)


def _rcp(v):
    y = pltpu.reciprocal(v, approx=True)
    return y * (2.0 - v * y)


def _inv_std(var):
    return _rcp(_rb(jnp.exp2(0.5 * jnp.log2(_rb(_rb(var) + EPS_B)))))


def _rsqrt_eps(var):
    return jnp.exp2(-0.5 * jnp.log2(var + EPS_B))


def _ln(v):
    d = v - jnp.mean(v, axis=-1, keepdims=True)
    return (d * _rsqrt_eps(jnp.mean(d * d, axis=-1, keepdims=True))).astype(bf16)


def _after(v):
    return jnp.where(v != v, jnp.uint32(1), jnp.uint32(0)) & jnp.uint32(0x10)


def _tie(p, v, dep):
    parts = [p[:8 * v]] if v else []
    parts.append(p[8 * v:8 * v + 8] | dep)
    if 8 * v + 8 < p.shape[0]:
        parts.append(p[8 * v + 8:])
    return jnp.concatenate(parts, axis=0) if len(parts) > 1 else parts[0]


def _phi(t):
    return jnp.where(t > 0, t + 1.0, jnp.exp(t))


def _nt_dot(a, b):
    return lax.dot_general(a, b, (((1,), (1,)), ((), ())), preferred_element_type=f32)


def _dot(a, b):
    return jnp.dot(a, b, preferred_element_type=f32)


def _wtile(ref, c, r0=0, nr=None):
    nr = ref.shape[1] if nr is None else nr
    return ref[c, r0:r0 + nr, :]


def _cols(ref, c0, n, r0=0, nr=None):
    return jnp.concatenate([_wtile(ref, c, r0, nr) for c in range(c0, c0 + n)], axis=1)


def _spread(deps, t0, t1):
    ties = {}
    for j, dep in enumerate(deps):
        when = t0 + (j * (t1 - t0)) // (len(deps) - 1)
        slot = ties.setdefault(when // 1024, {})
        key = (4 * ((when % 1024) // 512), (when % 512) // 16)
        slot[key] = dep if key not in slot else slot[key] | dep
    return ties


def _kernel(x_hbm, wq_hbm, wk_hbm, wv_hbm, wo_hbm, beta_hbm, wr_hbm, wg_hbm, wu_hbm, wd_hbm,
            out_hbm,
            xb, wq, wk, wv, wo, wg, wu, wd, beta_v, wr_v,
            xres, xn, qk, pqk, vT, o_s, SA, SB, MA, MB, Mst, Lst, AA, AB, xn2, r_s,
            hm_s, cm_s, gate_s, one_s, patch, stat_s, wr_s, zero_s, sems):
    def x_copy(s):
        r = pl.ds(pl.multiple_of(s * L, L), L)
        return pltpu.make_async_copy(x_hbm.at[r], xb.at[r], sems.at[s])

    def w_copies(src, dst, sem, c0=0, c1=None):
        c1 = dst.shape[0] if c1 is None else c1
        return [pltpu.make_async_copy(src.at[:, pl.ds(128 * c, 128)], dst.at[c], sems.at[sem])
                for c in range(c0, c1)]

    def start(copies):
        for c in copies:
            c.start()

    def wait(copies):
        for c in copies:
            c.wait()

    beta_c = pltpu.make_async_copy(beta_hbm, beta_v, sems.at[4])
    wr_c = pltpu.make_async_copy(wr_hbm, wr_v, sems.at[4])
    wq_lo, wq_mid, wq_hi = w_copies(wq_hbm, wq, 5, 0, 2), w_copies(wq_hbm, wq, 19, 2, 5), w_copies(wq_hbm, wq, 6, 5, 8)
    wk_c, wv_c, wo_c = w_copies(wk_hbm, wk, 7), w_copies(wv_hbm, wv, 8), w_copies(wo_hbm, wo, 9)
    mlp_c = w_copies(wg_hbm, wg, 10) + w_copies(wu_hbm, wu, 10) + w_copies(wd_hbm, wd, 10)

    def x0_copy(h):
        r = pl.ds(h * (L // 2), L // 2)
        return pltpu.make_async_copy(x_hbm.at[r], xb.at[r], sems.at[17 + h])

    beta_c.start()
    wr_c.start()
    x0_copy(0).start()
    x0_copy(1).start()
    start(wq_lo)
    start(wq_mid)
    start(wq_hi)
    start(wk_c)
    x_copy(1).start()
    start(wv_c)
    x_copy(2).start()
    x_copy(3).start()

    zero_s[0] = 0
    lane8 = lax.broadcasted_iota(jnp.int32, (8, 128), 1)
    for h in range(4):
        hm_s[h] = jnp.where((lane8 >= 32 * h) & (lane8 < 32 * h + 32), jnp.uint32(0xFFFFFFFF), jnp.uint32(0))
    ki = lax.broadcasted_iota(jnp.int32, (128, 128), 0)
    qi = lax.broadcasted_iota(jnp.int32, (128, 128), 1)
    cm_s[...] = jnp.where(ki <= qi, 0.0, NEG).astype(f32)
    row16 = lax.broadcasted_iota(jnp.int32, (16, 128), 0)
    one_s[...] = _pack(jnp.where(row16 == 0, 1.0, 0.0).astype(bf16))

    def setup_small():
        beta_c.wait()
        wr_c.wait()
        gate_row = jnp.broadcast_to(jax.nn.sigmoid(beta_v[...].astype(f32).reshape(1, H)), (8, H))
        lane_h = lax.broadcasted_iota(jnp.int32, (8, H), 1)
        for h in range(H):
            gh = jnp.sum(jnp.where(lane_h == h, gate_row, 0.0), axis=-1, keepdims=True)
            gate_s[h] = jnp.broadcast_to(gh, (8, 128))
        wr_s[...] = wr_v[...].astype(f32).reshape(1, D)

    def first_ln(s, dst, chunks=range(L // 16)):
        xsub = xb.at[pl.ds(s * L, L)]
        rsub = xres.at[pl.ds(s * L, L)]
        nsub = dst.at[pl.ds(s * (L // 2), L // 2)]
        deps = []
        for j in chunks:
            v = xsub[j * 16:(j + 1) * 16, :].astype(f32)
            rsub[j * 16:(j + 1) * 16, :] = v
            n = _pack(_ln(v))
            nsub[j * 8:(j + 1) * 8, :] = n
            deps.append(_after(pltpu.bitcast(n[:, 896:1024], f32)))
        return deps

    def out_copy(b):
        return pltpu.make_async_copy(xb.at[pl.ds(b * BR, BR)], out_hbm.at[pl.ds(b * BR, BR)], sems.at[11 + b])

    def proj_piece(src, s, w_ref, c, ties=None):
        xs = src.at[pl.ds(pl.multiple_of(s * (L // 2), L // 2), L // 2)]
        ps = [xs[:, 128 * g:128 * (g + 1)] for g in range(G)]
        for (g, v), dep in (ties or {}).items():
            ps[g] = _tie(ps[g], v, dep)
        return _dot(jnp.concatenate([_unpack(p) for p in ps], axis=1), _wtile(w_ref, c))

    def qkv(src, s, hooks=None):
        r0 = pl.multiple_of(s * (L // 2), L // 2)
        ties = {}
        n = 0
        for which, w_ref in ((0, wq), (1, wk), (2, wv)):
            for g in range(G):
                if hooks and n in hooks:
                    ties = hooks[n]() or ties
                y = proj_piece(src, s, w_ref, g, ties.get(n))
                if which < 2:
                    qk.at[which, g, pl.ds(r0, L // 2)][...] = _pack(((y * QSCALE) if which == 0 else y).astype(bf16))
                    pqk.at[which, g, pl.ds(r0, L // 2)][...] = _pack(_phi(y).astype(bf16))
                else:
                    vT.at[g, s][...] = _pack(y.astype(bf16).T)
                n += 1

    def step(i_qk, i_sm, Sw, Mw, Sr, Mr, filler=None, mem_read=True, mem_write=True):
        if i_qk is not None:
            gq = pl.multiple_of(i_qk % G, NI)
            rq = pl.multiple_of((i_qk // G) * (L // 2), L // 2)
            q_q = qk.at[0, pl.ds(gq, NI), pl.ds(rq, L // 2)]
            q_k = qk.at[1, pl.ds(gq, NI), pl.ds(rq, L // 2)]
        if i_sm is not None:
            gs = pl.multiple_of(i_sm % G, NI)
            ss = i_sm // G
            rs = pl.multiple_of(ss * (L // 2), L // 2)
            s_pq = pqk.at[0, pl.ds(gs, NI), pl.ds(rs, L // 2)]
            s_pk = pqk.at[1, pl.ds(gs, NI), pl.ds(rs, L // 2)]
            s_v = vT.at[pl.ds(gs, NI), ss]
            s_o = o_s.at[pl.ds(gs, NI), pl.ds(rs, L // 2)]
            s_M = Mst.at[pl.ds(gs, NI)]
            s_L = Lst.at[pl.ds(gs, NI)]
            s_g = gate_s.at[pl.ds(4 * gs, 4 * NI)]
        M, O, LS, REC, UPD = {}, {}, {}, {}, {}

        def put_scores(j, t, h, kt, sc):
            Sw.at[40 * j + TIDX[t, h, kt]][...] = sc
            mm = jnp.max(sc.reshape(16, 8, 128), axis=0)
            M[j, t, h] = jnp.maximum(M[j, t, h], mm) if (j, t, h) in M else mm

        def qk_tile(j, t, h, kt):
            kk = q_k[j, 64 * kt:64 * kt + 64, :]
            qu = q_q[j, 64 * t:64 * t + 64, :]
            if kt < t:
                put_scores(j, t, h, kt, _nt_dot(_unpack(kk & hm_s[h][0:1, :]), _unpack(qu)))
            elif h % 2 == 0:
                m0, m1 = hm_s[h][0:1, :], hm_s[h + 1][0:1, :]
                top = _nt_dot(_unpack(jnp.concatenate([kk[0:32] & m0, kk[0:32] & m1], axis=0)), _unpack(qu))
                both = jnp.concatenate([qu[32:64] & m1, qu[32:64] & m0], axis=0)
                low = _nt_dot(_unpack(kk[32:64]), _unpack(both))
                put_scores(j, t, h, kt, jnp.concatenate([top[0:64], low], axis=0) + cm_s[...])
                put_scores(j, t, h + 1, kt,
                           jnp.concatenate([top[64:128], pltpu.roll(low, 64, 1)], axis=0) + cm_s[...])
            if kt == t:
                Mw.at[16 * j + 4 * t + h][...] = jnp.broadcast_to(
                    jnp.max(M[j, t, h], axis=0, keepdims=True), (8, 128))

        def sm_tile(j, t, h, kt):
            if h == 0 and kt == 0 and mem_read:
                pq = _unpack(s_pq[j, 64 * t:64 * t + 64, :])
                REC[t] = _nt_dot(_unpack(s_L[j]), pq)
            sc = Sr[40 * j + TIDX[t, h, kt]]
            m = Mr[16 * j + 4 * t + h]
            p = jnp.exp2(sc.reshape(16, 8, 128) - m[None]).reshape(128, 128)
            ls = jnp.sum(p.reshape(16, 8, 128), axis=0)
            vt = _unpack(s_v[j, 16 * h:16 * h + 16, 128 * kt:128 * kt + 128])
            o = _dot(vt, p.astype(bf16))
            if kt == 0:
                O[t, h] = o
                LS[t, h] = ls
            else:
                O[t, h] = O[t, h] + o
                LS[t, h] = LS[t, h] + ls
            if kt == t:
                gt = s_g[4 * j + h][0:1, :]
                c2 = (1.0 - gt) * _rcp(jnp.sum(LS[t, h], axis=0, keepdims=True))
                O[t, h] = O[t, h] * c2
            if kt == t and h == 3:
                if mem_read:
                    rec = REC[t]
                    rden = _rcp(rec[128:136] + 1e-6)
                    rows = [rec[32 * hh:32 * hh + 32] * (s_g[4 * j + hh][0:1, :] * rden[hh:hh + 1, :]) + O[t, hh]
                            for hh in range(4)]
                else:
                    rows = [O[t, hh] for hh in range(4)]
                ot = jnp.concatenate(rows, axis=0).astype(bf16)
                s_o.at[j, pl.ds(64 * t, 64)][...] = _pack(ot.T)

        def mem_update_start(j):
            lhs = jnp.concatenate(
                [_unpack(s_v[j]), jnp.concatenate([_unpack(one_s[...])] * 4, axis=1)], axis=0)
            upd = _dot(lhs, _unpack(s_pk[j]))
            mn = (s_M[j] + upd[0:136]) if mem_read else upd[0:136]
            s_M.at[j][...] = mn
            hmask = jnp.concatenate([hm_s[hh] for hh in range(4) for _ in range(4)], axis=0)
            mb = pltpu.bitcast(pltpu.bitcast(mn[0:128], u32) & hmask, f32)
            sub = lax.broadcasted_iota(jnp.int32, (16, 128), 0)
            lane = lax.broadcasted_iota(jnp.int32, (16, 128), 1)
            z = jnp.broadcast_to(mn[128:129], (16, 128))
            zb = jnp.where(lane // 32 == sub, z, 0.0)
            UPD[j] = _pack(jnp.concatenate([mb, zb], axis=0).astype(bf16))

        work = [(j, x) for j in range(NI) for x in TILES]
        n_sm = 0
        for n, (j, x) in enumerate(work):
            if i_sm is not None:
                target = len(work) if i_qk is None else min(len(work), ((n + 1) * len(work)) // (len(work) - SKEW) + 1)
                target = n + 1 if i_qk is None else target
                while n_sm < target:
                    js, xs_ = work[n_sm]
                    if xs_ == TILES[0] and mem_write:
                        mem_update_start(js)
                    sm_tile(js, *xs_)
                    if xs_ == TILES[-1] and mem_write:
                        s_L.at[js][...] = UPD[js]
                    n_sm += 1
            if i_qk is not None:
                qk_tile(j, *x)
            if filler is not None:
                filler(n + 1, len(work))

    def oproj_piece(b, A, c, ties=None):
        osub = o_s.at[:, pl.ds(pl.multiple_of(b * (BR // 2), BR // 2), BR // 2)]
        ps = [osub[g] for g in range(G)]
        for (g, v), dep in (ties or {}).items():
            ps[g] = _tie(ps[g], v, dep)
        o = jnp.concatenate([_unpack(p) for p in ps], axis=1)
        A[:, 128 * c:128 * (c + 1)] = _dot(o, _wtile(wo, c))

    def epilogue_refs(b):
        return (xres.at[pl.ds(pl.multiple_of(b * BR, BR), BR)],
                xb.at[pl.ds(pl.multiple_of(b * BR, BR), BR)],
                xn2.at[pl.ds(pl.multiple_of(b * (BR // 2), BR // 2), BR // 2)],
                xn.at[pl.ds(pl.multiple_of(b * (BR // 2), BR // 2), BR // 2)])

    def epi1(refs, A, j, base, racc):
        xr, _, n2r, _ = refs
        rows = slice(j * 16, (j + 1) * 16)
        x1 = xr[rows, :] + A[rows, :]
        mean = jnp.mean(x1, axis=-1, keepdims=True)
        d = x1 - mean
        var = jnp.mean(d * d, axis=-1, keepdims=True)
        inv = _inv_std(var)
        n2 = d * inv
        n2r[j * 8:(j + 1) * 8, :] = _pack(n2.astype(bf16))
        r = jnp.sum(n2 * wr_s[...], axis=-1, keepdims=True)
        lane = lax.broadcasted_iota(jnp.int32, (8, 128), 1)
        racc = jnp.where(lane == base + 2 * j, r[0:8], racc)
        racc = jnp.where(lane == base + 2 * j + 1, r[8:16], racc)
        grow = 1.0 + inv
        scale2 = grow * _rsqrt_eps(var * (grow * grow))
        done = _after(jnp.broadcast_to(r[0:8] + r[8:16], (8, 128)))
        return x1, mean, d, scale2, n2, racc, done

    def epi2(refs, j, x1, d, scale2, n2, last):
        xr, xo, _, n1r = refs
        rows = slice(j * 16, (j + 1) * 16)
        x2 = x1 + n2
        xr[rows, :] = x2
        if last:
            xo[rows, :] = x2.astype(bf16)
            return _after(x2[0:8, 896:1024])
        n1 = _pack((d * scale2).astype(bf16))
        n1r[j * 8:(j + 1) * 8, :] = n1
        return _after(pltpu.bitcast(n1[:, 896:1024], f32)) | _after(x2[0:8, 896:1024])

    def put_scores(b, racc):
        half = b // 2

        @pl.when(b % 2 == 0)
        def _():
            r_s[half] = racc

        @pl.when(b % 2 == 1)
        def _():
            r_s[half] = r_s[half] + racc

    def oproj_epilogue(b, A, bn, An, last):
        refs = epilogue_refs(b)
        racc = jnp.zeros((8, 128), f32)
        deps = []
        for j in range(BR // 16):
            x1, _, d, scale2, n2, racc, done = epi1(refs, A, j, (b % 2) * (BR // 8), racc)
            deps.append(done | epi2(refs, j, x1, d, scale2, n2, last))
        ties = _spread(deps, TIE0, TIE1)
        for c in range(G):
            oproj_piece(bn, An, c, ties.get(c))
        put_scores(b, racc)

    def layer(l):
        first, last = l == 0, l == NLAYERS - 1

        with jax.named_scope("P_qkv"):
            if first:
                bufs = (xn, xn2)
                x0_copy(0).wait()
                first_ln(0, bufs[0], range(0, L // 32))
                x0_copy(1).wait()
                first_ln(0, bufs[0], range(L // 32, L // 16))
                setup_small()
                wait(wq_lo)

                def before_v0():
                    wait(wv_c)
                    x_copy(1).wait()
                    return _spread(first_ln(1, bufs[1]), 16 * 1024 + 600, 24 * 1024 - 100)

                qkv(bufs[0], 0, {2: lambda: wait(wq_mid), 5: lambda: wait(wq_hi), 8: lambda: wait(wk_c), 16: before_v0})
                for s in range(1, NSEG):
                    def before(s=s):
                        if s == 1:
                            start(wo_c)
                            start(mlp_c)
                        if s + 1 < NSEG:
                            x_copy(s + 1).wait()
                            return _spread(first_ln(s + 1, bufs[(s + 1) % 2]), 600, 16 * 1024)

                    qkv(bufs[s % 2], s, {0: before})
            else:
                lax.fori_loop(0, NSEG, lambda s, _: qkv(xn, s), None)

        nstep = 4 * G // NI
        per_seg = G // NI
        sets = ((SA, MA), (SB, MB))

        def att_step(i, **kw):
            step((i + 1) * NI, i * NI, *sets[i % 2], *sets[1 - i % 2], **kw)

        def block(fn):
            pl.when(zero_s[0] == 0)(fn)

        with jax.named_scope("P_att"):
            step(0, None, SB, MB, None, None)
            for i in range(per_seg):
                block(lambda i=i: att_step(i, mem_read=False))

            def att_body(i, _):
                @pl.when(i % 2 == 0)
                def _():
                    step((i + 1) * NI, i * NI, SA, MA, SB, MB)

                @pl.when(i % 2 == 1)
                def _():
                    step((i + 1) * NI, i * NI, SB, MB, SA, MA)

            lax.fori_loop(per_seg, nstep - per_seg, att_body, None)
            for i in range(nstep - per_seg, nstep - 1):
                block(lambda i=i: att_step(i, mem_write=False))

        if first:
            wait(wo_c)

        def filler(n, total):
            if n % (total // G) == 0:
                oproj_piece(0, AA, n // (total // G) - 1)

        with jax.named_scope("P_op"):
            if (nstep - 1) % 2 == 0:
                step(None, (nstep - 1) * NI, None, None, SB, MB, filler, mem_write=False)
            else:
                step(None, (nstep - 1) * NI, None, None, SA, MA, filler, mem_write=False)

            def op_body(i, _):
                if last:
                    @pl.when(i >= 2)
                    def _():
                        out_copy(i - 2).start()

                @pl.when(i % 2 == 1)
                def _():
                    oproj_epilogue(i - 1, AA, i, AB, last)

                @pl.when(i % 2 == 0)
                def _():
                    oproj_epilogue(i - 1, AB, i, AA, last)

            lax.fori_loop(1, NB, op_body, None)

        if last:
            out_copy(NB - 2).start()

        with jax.named_scope("P_tail"):
            with jax.named_scope("T_epi1"):
                refs = epilogue_refs(NB - 1)
                A_last = AB if (NB - 1) % 2 == 1 else AA
                racc = jnp.zeros((8, 128), f32)
                for j in range(BR // 16):
                    x1, mean, d, scale2, n2, racc, _ = epi1(refs, A_last, j, ((NB - 1) % 2) * (BR // 8), racc)
                    if last:
                        epi2(refs, j, x1, d, scale2, n2, True)
                    else:
                        A_last[j * 16:(j + 1) * 16, :] = x1
                        stat_s.at[0][j * 16:(j + 1) * 16, :] = jnp.broadcast_to(mean, (16, 128))
                        stat_s.at[1][j * 16:(j + 1) * 16, :] = jnp.broadcast_to(scale2, (16, 128))
            r_all = jnp.concatenate([r_s[0], r_s[1] + racc], axis=0)
            if last:
                out_copy(NB - 1).start()
            if first:
                wait(mlp_c)

            with jax.named_scope("T_top2"):
                rr = pltpu.bitcast(_rb(r_all), u32)
                sub = lax.broadcasted_iota(jnp.int32, (16, 128), 0)
                lane = lax.broadcasted_iota(jnp.int32, (16, 128), 1)
                pos = ((sub // 8) * 1024 + lane * 8 + (sub % 8)).astype(u32)
                neg = (rr >> 31) == 1
                key = pltpu.bitcast(rr | jnp.where(neg, pos, (S - 1) - pos), f32)

                def top(k):
                    return jnp.max(jnp.max(k, axis=1, keepdims=True), axis=0, keepdims=True)

                k1 = top(key)
                k2 = top(jnp.where(key == k1, -jnp.inf, key))

                def decode(k):
                    kb = pltpu.bitcast(jnp.broadcast_to(k, (8, 128)), u32)
                    code = kb & jnp.uint32(S - 1)
                    p = jnp.where((kb >> 31) == 1, code, (S - 1) - code).astype(jnp.int32)
                    score = pltpu.bitcast(kb & jnp.uint32(0xFFFF0000), f32)
                    return jnp.clip(jnp.max(p), 0, S - 1), score

                i1, m1 = decode(k1)
                i2, m2 = decode(k2)

            with jax.named_scope("T_pick"):
                row = lax.broadcasted_iota(jnp.int32, (16, D), 0)

                def pick(i):
                    blk = _unpack(xn2[pl.ds(pl.multiple_of((i // 16) * 8, 8), 8), :]).astype(f32)
                    return jnp.sum(jnp.where(row == i % 16, blk, 0.0), axis=0, keepdims=True)

                xs = jnp.where(row == 0, pick(i1), jnp.where(row == 1, pick(i2), 0.0)).astype(bf16)

            with jax.named_scope("T_mlp"):
                ties = {}
                if not last:
                    for j in range(BR // 16):
                        rows = slice(j * 16, (j + 1) * 16)
                        x1 = A_last[rows, :]
                        n2 = _unpack(refs[2][j * 8:(j + 1) * 8, :]).astype(f32)
                        done = epi2(refs, j, x1, x1 - stat_s[0, rows, 0:1], stat_s[1, rows, 0:1], n2, False)
                        key_ = 3 + (j * (2 * NC - 3)) // (BR // 16)
                        ties[key_] = done if key_ not in ties else ties[key_] | done

                def weights(w_ref, c, key_):
                    tiles = [_pack(_wtile(w_ref, 4 * c + t)) for t in range(4)] if key_ in ties else None
                    if tiles is None:
                        return _cols(w_ref, 4 * c, 4)
                    tiles[0] = _tie(tiles[0], 0, ties[key_])
                    return jnp.concatenate([_unpack(t) for t in tiles], axis=1)

                def gate_up(c):
                    gg = _rb(_dot(xs, weights(wg, c, 2 * c)))
                    uu = _rb(_dot(xs, weights(wu, c, 2 * c + 1)))
                    return (_rb(gg * jax.nn.sigmoid(gg)) * uu).astype(bf16)

                y = jnp.zeros((16, D), f32)
                a = gate_up(0)
                for c in range(NC):
                    a_next = gate_up(c + 1) if c + 1 < NC else None
                    y = y + _dot(a, _cols(wd, 0, G, c * FC, FC))
                    a = a_next
                row8 = lax.broadcasted_iota(jnp.int32, (16, 128), 0)
                gsel = _rb(jax.nn.sigmoid(jnp.where(row8 == 0, m1[0:1, :], m2[0:1, :])))
                upd = _rb(_rb(y) * jnp.concatenate([gsel] * (D // 128), axis=1))

            with jax.named_scope("T_fix"):
                def rows_at(i):
                    return pl.multiple_of((i // 16) * 16, 16)

                def updated(i0):
                    xv = xres[pl.ds(rows_at(i0), 16), :]
                    for i, j in ((i1, 0), (i2, 1)):
                        hit = (row == i % 16) & (i // 16 == i0 // 16)
                        xv = xv + jnp.where(hit, upd[j:j + 1, :], 0.0)
                    return xv.astype(bf16)

                xv1, xv2 = updated(i1), updated(i2)
                if last:
                    patch[0] = xv1
                    patch[1] = xv2
                    for b in range(NB):
                        out_copy(b).wait()
                    b1, b2 = rows_at(i1), rows_at(i2)
                    c1 = pltpu.make_async_copy(patch.at[0], out_hbm.at[pl.ds(b1, 16)], sems.at[15])
                    c2 = pltpu.make_async_copy(patch.at[1], out_hbm.at[pl.ds(b2, 16)], sems.at[16])

                    @pl.when(b1 != b2)
                    def _():
                        c1.start()

                    c2.start()

                    @pl.when(b1 != b2)
                    def _():
                        c1.wait()

                    c2.wait()
                else:
                    n1, n2 = _pack(_ln(xv1.astype(f32))), _pack(_ln(xv2.astype(f32)))
                    for i, xv, nn in ((i1, xv1, n1), (i2, xv2, n2)):
                        xres[pl.ds(rows_at(i), 16), :] = xv.astype(f32)
                        xn.at[pl.ds(pl.multiple_of((i // 16) * 8, 8), 8)][...] = nn

    for l in range(NLAYERS):
        layer(l)


@jax.jit
def pallas_interleave_layers__memory_aug_infini_attn__moe_arch_mod__prompt_kernel(
    A_x, A_wq, A_wk, A_wv, A_wo, A_beta, B_x, B_w_r, B_w_gate, B_w_up, B_w_down,
):
    del B_x
    x = A_x.reshape(S, D)
    hbm = pl.BlockSpec(memory_space=pltpu.HBM)
    scratch = [
        pltpu.VMEM((S, D), bf16),
        pltpu.VMEM((D // 128, D, 128), bf16),
        pltpu.VMEM((D // 128, D, 128), bf16),
        pltpu.VMEM((D // 128, D, 128), bf16),
        pltpu.VMEM((D // 128, D, 128), bf16),
        pltpu.VMEM((F // 128, D, 128), bf16),
        pltpu.VMEM((F // 128, D, 128), bf16),
        pltpu.VMEM((D // 128, F, 128), bf16),
        pltpu.VMEM((H,), bf16),
        pltpu.VMEM((D,), bf16),
        pltpu.VMEM((S, D), f32),
        pltpu.VMEM((S // 2, D), u32),
        pltpu.VMEM((2, G, S // 2, 128), u32),
        pltpu.VMEM((2, G, S // 2, 128), u32),
        pltpu.VMEM((G, NSEG, 64, L), u32),
        pltpu.VMEM((G, S // 2, 128), u32),
        pltpu.VMEM((40 * NI, 128, 128), f32),
        pltpu.VMEM((40 * NI, 128, 128), f32),
        pltpu.VMEM((16 * NI, 8, 128), f32),
        pltpu.VMEM((16 * NI, 8, 128), f32),
        pltpu.VMEM((G, 136, 128), f32),
        pltpu.VMEM((G, 72, 128), u32),
        pltpu.VMEM((BR, D), f32),
        pltpu.VMEM((BR, D), f32),
        pltpu.VMEM((S // 2, D), u32),
        pltpu.VMEM((2, 8, 128), f32),
        pltpu.VMEM((4, 8, 128), u32),
        pltpu.VMEM((128, 128), f32),
        pltpu.VMEM((H, 8, 128), f32),
        pltpu.VMEM((8, 128), u32),
        pltpu.VMEM((2, 16, D), bf16),
        pltpu.VMEM((2, BR, 128), f32),
        pltpu.VMEM((1, D), f32),
        pltpu.SMEM((1,), jnp.int32),
        pltpu.SemaphoreType.DMA((20,)),
    ]
    out = pl.pallas_call(
        _kernel,
        out_shape=jax.ShapeDtypeStruct((S, D), bf16),
        in_specs=[hbm] * 10,
        out_specs=hbm,
        scratch_shapes=scratch,
        compiler_params=pltpu.CompilerParams(vmem_limit_bytes=124 * 1024 * 1024),
        name="infini_mod_kernel",
    )(x, A_wq, A_wk, A_wv, A_wo, A_beta, B_w_r, B_w_gate, B_w_up, B_w_down)
    return out.reshape(1, S, D)
```
